```python
import jax
import jax.numpy as jnp

def _softmax(x, axis=-1):
    return jax.nn.softmax(x, axis=axis)

def _gelu(x):
    return jax.nn.gelu(x, approximate=True)

def _silu(x):
    return jax.nn.silu(x)

def _sigmoid(x):
    return jax.nn.sigmoid(x)

def _layernorm(x, axis=-1, eps=1e-05):
    m = jnp.mean(x, axis=axis, keepdims=True)
    v = jnp.var(x, axis=axis, keepdims=True)
    return (x - m) / jnp.sqrt(v + eps)

def _scatter_add(tgt, idx, src, axis=0):
    return tgt.at[idx].add(src)

def _segment_sum(src, seg, n):
    return jax.ops.segment_sum(src, seg, n)

class _Rng:

    def __init__(self, key):
        self._k = key

    def _next(self):
        self._k, sub = jax.random.split(self._k)
        return sub

    def normal(self, shape):
        return jax.random.normal(self._next(), shape, dtype=jnp.bfloat16)

    def randint(self, lo, hi, shape):
        return jax.random.randint(self._next(), shape, lo, hi, dtype=jnp.int32)

    def uniform(self, shape, lo=0.0, hi=1.0):
        return jax.random.uniform(self._next(), shape, jnp.bfloat16, lo, hi)

    def permutation(self, n):
        return jax.random.permutation(self._next(), n)
kernel_name = 'adaLN_cond__compressed_kv_cla__mixer_s_mlp__prompt'

def setup_inputs():
    _rng = _Rng(jax.random.key(int.from_bytes(__import__("os").urandom(4), "little")))
    _w = lambda a: (lambda t: t.astype(jnp.bfloat16) if jnp.issubdtype(t.dtype, jnp.floating) else t)(jnp.asarray(a))

    def _A_setup():
        B, H, Sq, Sk, D, M = (1, 32, 2048, 2048, 128, 640)
        Dc = 4 * D
        return {'x': _w((lambda *s: _rng.normal(s) * 0.05)(B, Sq, M)), 'c_kv': _w((lambda *s: _rng.normal(s) * 0.05)(B, Sk, Dc)), 'w_q': _w((lambda *s: _rng.normal(s) * 0.05)(M, H, D) * M ** (-0.5)), 'w_uk': _w((lambda *s: _rng.normal(s) * 0.05)(Dc, H, D) * Dc ** (-0.5)), 'w_uv': _w((lambda *s: _rng.normal(s) * 0.05)(Dc, H, D) * Dc ** (-0.5)), 'w_o': _w((lambda *s: _rng.normal(s) * 0.05)(H, D, M) * (H * D) ** (-0.5))}
    _A_in = _A_setup()

    def _B_setup():
        B, S, D, F = (1, 2048, 640, 1728)
        return {'x': _w((lambda *s: _rng.normal(s) * 0.05)(B, S, D)), 'w1': _w((lambda *s: _rng.normal(s) * 0.05)(D, D) * D ** (-0.5)), 'w2': _w((lambda *s: _rng.normal(s) * 0.05)(D, D) * D ** (-0.5)), 'w3': _w((lambda *s: _rng.normal(s) * 0.05)(D, F) * D ** (-0.5)), 'w4': _w((lambda *s: _rng.normal(s) * 0.05)(F, D) * F ** (-0.5))}
    _B_in = _B_setup()
    return {'A_x': _A_in['x'], 'A_c_kv': _A_in['c_kv'], 'A_w_q': _A_in['w_q'], 'A_w_uk': _A_in['w_uk'], 'A_w_uv': _A_in['w_uv'], 'A_w_o': _A_in['w_o'], 'B_x': _B_in['x'], 'B_w1': _B_in['w1'], 'B_w2': _B_in['w2'], 'B_w3': _B_in['w3'], 'B_w4': _B_in['w4'], 'c': _w((lambda *s: _rng.normal(s) * 0.05)(1, 640)), 'w_mod': _w((lambda *s: _rng.normal(s) * 0.05)(640, 6 * 640) * 640 ** (-0.5))}

def reference(A_x, A_c_kv, A_w_q, A_w_uk, A_w_uv, A_w_o, B_x, B_w1, B_w2, B_w3, B_w4, c, w_mod):

    def _A_ref(x, c_kv, w_q, w_uk, w_uv, w_o):
        B, Sq, M = (x.shape[0], x.shape[1], x.shape[2])
        Sk = c_kv.shape[1]
        H, D = (w_q.shape[1], w_q.shape[2])
        q = jnp.einsum('bqm,mhd->bhqd', x, w_q)
        k = jnp.einsum('bkc,chd->bhkd', c_kv, w_uk)
        v = jnp.einsum('bkc,chd->bhkd', c_kv, w_uv)
        scores = jnp.einsum('bhqd,bhkd->bhqk', q, k) * D ** (-0.5)
        off = Sk - Sq
        qi = jnp.arange(Sq)[:, None]
        kj = jnp.arange(Sk)[None, :]
        cmask = kj <= qi + off
        scores = jnp.where(cmask[None, None], scores, -1000000000.0)
        p = _softmax(scores, axis=-1)
        ctx = jnp.einsum('bhqk,bhkd->bhqd', p, v)
        return jnp.einsum('bhqd,hdm->bqm', ctx, w_o)

    def _B_ref(x, w1, w2, w3, w4):
        B, S, D = x.shape
        h = _gelu(_layernorm(x, axis=-1) @ w1)
        c = D // 4
        g0 = jnp.pad(h[:, :, 0 * c:1 * c], ((0, 0), (1, 0), (0, 0)))[:, :S, :]
        g1 = jnp.pad(h[:, :, 1 * c:2 * c], ((0, 0), (0, 1), (0, 0)))[:, 1:, :]
        g2 = jnp.pad(h[:, :, 2 * c:3 * c], ((0, 0), (2, 0), (0, 0)))[:, :S, :]
        g3 = jnp.pad(h[:, :, 3 * c:], ((0, 0), (0, 2), (0, 0)))[:, 2:, :]
        hs = jnp.concatenate([g0, g1, g2, g3], axis=-1) @ w2
        x1 = x + hs
        h2 = _gelu(_layernorm(x1, axis=-1) @ w3) @ w4
        return x1 + h2
    x = A_x
    mod = (_silu(c) @ w_mod).reshape(c.shape[0], 6, 1, -1)
    sa, ca, ga, sb, cb, gb = (mod[:, 0].copy(), mod[:, 1].copy(), mod[:, 2].copy(), mod[:, 3].copy(), mod[:, 4].copy(), mod[:, 5].copy())
    h = _layernorm(x, axis=-1) * (1 + ca) + sa
    x = x + ga * _A_ref(h, A_c_kv, A_w_q, A_w_uk, A_w_uv, A_w_o)
    h = _layernorm(x, axis=-1) * (1 + cb) + sb
    x = x + gb * _B_ref(h, B_w1, B_w2, B_w3, B_w4)
    return x
```

```python
import functools
import numpy as np
import jax
import jax.numpy as jnp
from jax import lax
import jax.experimental.pallas as pl
import jax.experimental.pallas.tpu as pltpu

S = 2048; M = 640; H = 32; D = 128; DC = 512; F = 1728
BQ = 256
LOG2E = 1.4426950408889634
QSCALE = float(D ** -0.5) * LOG2E
f32 = jnp.float32; bf16 = jnp.bfloat16
NEG = -1e30


def _ln(x):
    m = jnp.mean(x, axis=-1, keepdims=True)
    xc = x - m
    v = jnp.mean(xc * xc, axis=-1, keepdims=True)
    return xc * lax.rsqrt(v + 1e-5)


def _gelu(x):
    c0 = float(np.sqrt(2.0 / np.pi))
    u = c0 * (x + 0.044715 * (x * x * x))
    return 0.5 * x * (1.0 + jnp.tanh(u))


def _dot(a, b):
    return jnp.dot(a, b, preferred_element_type=f32)


def _kernel(x_hbm, ckv_hbm, wq_ref, wuk_ref, wuv_ref, wo_hbm, w1_hbm, w2_hbm, w3_hbm, w4_hbm, c_ref, wmod_hbm,
            out_hbm,
            x_s, ckv_s, hmod_s, wmod_s, mod_s, wo_s, w1_s, w2_s, w3_s, w4_s,
            q_s, kT_s, v_s, S_s, ctx_s, h_s, h1_s, x2_s, out_s, sems):
    h = pl.program_id(0)

    cp_x = pltpu.make_async_copy(x_hbm, x_s, sems.at[0])
    cp_ckv = pltpu.make_async_copy(ckv_hbm, ckv_s, sems.at[1])
    cp_wmod = pltpu.make_async_copy(wmod_hbm, wmod_s, sems.at[2])
    cp_wo = pltpu.make_async_copy(wo_hbm, wo_s, sems.at[3])
    cp_w1 = pltpu.make_async_copy(w1_hbm, w1_s, sems.at[4])
    cp_w2 = pltpu.make_async_copy(w2_hbm, w2_s, sems.at[5])
    cp_w3 = pltpu.make_async_copy(w3_hbm, w3_s, sems.at[6])
    cp_w4 = pltpu.make_async_copy(w4_hbm, w4_s, sems.at[7])
    cp_out = pltpu.make_async_copy(out_s, out_hbm, sems.at[8])

    @pl.when(h == 0)
    def _prologue():
        cp_ckv.start(); cp_wmod.start(); cp_x.start()
        cp_wo.start(); cp_w1.start(); cp_w2.start(); cp_w3.start(); cp_w4.start()
        cp_wmod.wait()
        c = c_ref[...].astype(f32)
        sc = c * (1.0 / (1.0 + jnp.exp(-c)))
        sc8 = jnp.broadcast_to(sc, (16, M)).astype(bf16)
        mod = _dot(sc8, wmod_s[...])
        mod_s[...] = mod[0:8, :]
        cp_x.wait()
        sa = mod_s[0:1, 0:M]
        ca = mod_s[0:1, M:2 * M]

        def ln_body(i, carry):
            r = pl.ds(pl.multiple_of(i * 256, 256), 256)
            xb = x_s[r, :].astype(f32)
            hb = _ln(xb) * (1.0 + ca) + sa
            hmod_s[r, :] = hb.astype(bf16)
            return carry
        lax.fori_loop(0, S // 256, ln_body, 0)
        cp_ckv.wait()

    q_s[...] = (_dot(hmod_s[...], wq_ref[...]) * QSCALE).astype(bf16)
    kk = _dot(ckv_s[...], wuk_ref[...])
    kT_s[...] = kk.T.astype(bf16)
    v_s[...] = _dot(ckv_s[...], wuv_ref[...]).astype(bf16)

    row = lax.broadcasted_iota(jnp.int32, (BQ, BQ), 0)
    col = lax.broadcasted_iota(jnp.int32, (BQ, BQ), 1)
    causal = col <= row

    for i in range(S // BQ):
        q_i = q_s[i * BQ:(i + 1) * BQ, :]
        nkv = i + 1
        m = None
        for j in range(nkv):
            s = _dot(q_i, kT_s[:, j * BQ:(j + 1) * BQ])
            if j == i:
                s = jnp.where(causal, s, NEG)
            S_s[:, j * BQ:(j + 1) * BQ] = s
            for t in range(BQ // 128):
                st = s[:, t * 128:(t + 1) * 128]
                m = st if m is None else jnp.maximum(m, st)
        m = jnp.max(m, axis=-1, keepdims=True)
        mb = jnp.broadcast_to(m, (BQ, 128))
        l = None
        acc = None
        for j in range(nkv):
            ps = []
            for t in range(BQ // 128):
                st = S_s[:, j * BQ + t * 128: j * BQ + (t + 1) * 128]
                p = jnp.exp2(st - mb)
                l = p if l is None else l + p
                ps.append(p.astype(bf16))
            pj = jnp.concatenate(ps, axis=1)
            o = _dot(pj, v_s[j * BQ:(j + 1) * BQ, :])
            acc = o if acc is None else acc + o
        l = jnp.sum(l, axis=-1, keepdims=True)
        ctx = acc * (1.0 / l)
        ctx_s[h, i * BQ:(i + 1) * BQ, :] = ctx.astype(bf16)

    @pl.when(h == H - 1)
    def _epilogue():
        cp_wo.wait(); cp_w1.wait(); cp_w2.wait(); cp_w3.wait(); cp_w4.wait()
        ga = mod_s[0:1, 2 * M:3 * M]
        sb = mod_s[0:1, 3 * M:4 * M]
        cb = mod_s[0:1, 4 * M:5 * M]
        gb = mod_s[0:1, 5 * M:6 * M]
        RB = 256
        h1_s[0:8, :] = jnp.zeros((8, M), f32)
        h1_s[S + 8:S + 16, :] = jnp.zeros((8, M), f32)

        def pass1(i, carry):
            r0 = pl.multiple_of(i * RB, RB)
            r = pl.ds(r0, RB)
            acc = None
            for hh in range(H):
                o = _dot(ctx_s[hh, r, :], wo_s[hh * D:(hh + 1) * D, :])
                acc = o if acc is None else acc + o
            x2 = x_s[r, :].astype(f32) + ga * acc
            x2_s[r, :] = x2
            hb = _ln(x2) * (1.0 + cb) + sb
            h_s[r, :] = hb
            g = _gelu(_dot(_ln(hb).astype(bf16), w1_s[...]))
            h1_s[pl.ds(r0 + 8, RB), :] = g
            return carry
        lax.fori_loop(0, S // RB, pass1, 0)

        lane = lax.broadcasted_iota(jnp.int32, (RB, 128), 1)

        def pass2(i, carry):
            r0 = pl.multiple_of(i * RB, RB)
            r = pl.ds(r0, RB)

            win = h1_s[pl.ds(r0, RB + 16), :]

            def sh(off, t):
                return win[8 + off:8 + off + RB, t * 128:(t + 1) * 128]
            t0 = sh(-1, 0)
            t1 = jnp.where(lane < 32, sh(-1, 1), sh(1, 1))
            t2 = jnp.where(lane < 64, sh(1, 2), sh(-2, 2))
            t3 = jnp.where(lane < 96, sh(-2, 3), sh(2, 3))
            t4 = sh(2, 4)
            g = jnp.concatenate([t0, t1, t2, t3, t4], axis=1).astype(bf16)
            x1 = h_s[r, :] + _dot(g, w2_s[...])
            u = _gelu(_dot(_ln(x1).astype(bf16), w3_s[...])).astype(bf16)
            h2 = _dot(u, w4_s[...])
            out = x2_s[r, :] + gb * (x1 + h2)
            out_s[r, :] = out.astype(bf16)
            return carry
        lax.fori_loop(0, S // RB, pass2, 0)
        cp_out.start()
        cp_out.wait()


@jax.jit
def pallas_adaLN_cond__compressed_kv_cla__mixer_s_mlp__prompt_kernel(
        A_x, A_c_kv, A_w_q, A_w_uk, A_w_uv, A_w_o, B_x, B_w1, B_w2, B_w3, B_w4, c, w_mod):
    x = A_x.reshape(S, M)
    ckv = A_c_kv.reshape(S, DC)
    wq = A_w_q.reshape(M, H * D)
    wuk = A_w_uk.reshape(DC, H * D)
    wuv = A_w_uv.reshape(DC, H * D)
    wo = A_w_o.reshape(H * D, M)
    anyspec = pl.BlockSpec(memory_space=pl.ANY)
    out = pl.pallas_call(
        _kernel,
        grid=(H,),
        in_specs=[anyspec, anyspec,
                  pl.BlockSpec((M, D), lambda h: (0, h)),
                  pl.BlockSpec((DC, D), lambda h: (0, h)),
                  pl.BlockSpec((DC, D), lambda h: (0, h)),
                  anyspec, anyspec, anyspec, anyspec, anyspec,
                  pl.BlockSpec((1, M), lambda h: (0, 0)),
                  anyspec],
        out_specs=anyspec,
        out_shape=jax.ShapeDtypeStruct((S, M), bf16),
        scratch_shapes=[
            pltpu.VMEM((S, M), bf16),
            pltpu.VMEM((S, DC), bf16),
            pltpu.VMEM((S, M), bf16),
            pltpu.VMEM((M, 6 * M), bf16),
            pltpu.VMEM((8, 6 * M), f32),
            pltpu.VMEM((H * D, M), bf16),
            pltpu.VMEM((M, M), bf16),
            pltpu.VMEM((M, M), bf16),
            pltpu.VMEM((M, F), bf16),
            pltpu.VMEM((F, M), bf16),
            pltpu.VMEM((S, D), bf16),
            pltpu.VMEM((D, S), bf16),
            pltpu.VMEM((S, D), bf16),
            pltpu.VMEM((BQ, S), f32),
            pltpu.VMEM((H, S, D), bf16),
            pltpu.VMEM((S, M), f32),
            pltpu.VMEM((S + 16, M), f32),
            pltpu.VMEM((S, M), f32),
            pltpu.VMEM((S, M), bf16),
            pltpu.SemaphoreType.DMA((9,)),
        ],
        compiler_params=pltpu.CompilerParams(
            dimension_semantics=("arbitrary",),
            vmem_limit_bytes=110 * 1024 * 1024,
        ),
    )(x, ckv, wq, wuk, wuv, wo, B_w1, B_w2, B_w3, B_w4, c, w_mod)
    return out.reshape(1, S, M)
```

```python
import os
import numpy as np
import jax
import jax.numpy as jnp
from jax import lax
import jax.experimental.pallas as pl
import jax.experimental.pallas.tpu as pltpu

S = 2048; M = 640; H = 32; D = 128; DC = 512; F = 1728
BQ = int(os.environ.get("BQ", 128))
KC = int(os.environ.get("KC", 512))
PVC = int(os.environ.get("PVC", 512))
PR = int(os.environ.get("PR", 128))
PIPE = int(os.environ.get("PIPE", 1))
PDELAY = int(os.environ.get("PDELAY", 1))
RB = int(os.environ.get("RB", 256))
FLAGS = {k: True for k in os.environ.get("KFLAGS", "").split(",") if k} or None
LOG2E = 1.4426950408889634
QSCALE = float(D ** -0.5) * LOG2E
f32 = jnp.float32; bf16 = jnp.bfloat16
NEG = -1e30
NP = M // 128
NC = DC // 128


def _ln(x):
    m = jnp.mean(x, axis=-1, keepdims=True)
    xc = x - m
    v = jnp.mean(xc * xc, axis=-1, keepdims=True)
    return xc * lax.rsqrt(v + 1e-5)


def _gelu(x):
    c0 = float(np.sqrt(2.0 / np.pi))
    u = c0 * (x + 0.044715 * (x * x * x))
    return 0.5 * x * (1.0 + jnp.tanh(u))


def _dot(a, b):
    return jnp.dot(a, b, preferred_element_type=f32)


def _kernel(x_hbm, ckv_hbm, wq_hbm, wuk_hbm, wuv_hbm, wo_hbm, w1_hbm, w2_hbm, w3_hbm, w4_hbm, c_ref, wmod_hbm,
            out_hbm,
            x_s, ckv_s, hmod_s, wmod_s, mod_s, wo_s, w1_s, w2_s, w3_s, w4_s,
            wq_s, wuk_s, wuv_s,
            q_s, kT_s, v_s, h_s, h1_s, x2_s, out_s, sems, wsems):
    h = pl.program_id(0)
    slot = h % 2

    def pcopies(hh, sl):
        c0 = pl.multiple_of(hh * D, D)
        return [pltpu.make_async_copy(wq_hbm.at[:, pl.ds(c0, D)], wq_s.at[sl], wsems.at[0, sl]),
                pltpu.make_async_copy(wuk_hbm.at[:, pl.ds(c0, D)], wuk_s.at[sl], wsems.at[1, sl]),
                pltpu.make_async_copy(wuv_hbm.at[:, pl.ds(c0, D)], wuv_s.at[sl], wsems.at[2, sl])]

    def wocopy(hh, sl):
        return pltpu.make_async_copy(wo_hbm.at[pl.ds(pl.multiple_of(hh * D, D), D), :], wo_s.at[sl], wsems.at[3, sl])

    cp_x = pltpu.make_async_copy(x_hbm, x_s, sems.at[0])
    cp_ckv = [pltpu.make_async_copy(ckv_hbm.at[:, t * 128:(t + 1) * 128], ckv_s.at[t], sems.at[9 + t]) for t in range(NC)]
    cp_wmod = pltpu.make_async_copy(wmod_hbm, wmod_s, sems.at[2])
    cp_w1 = pltpu.make_async_copy(w1_hbm, w1_s, sems.at[4])
    cp_w2 = pltpu.make_async_copy(w2_hbm, w2_s, sems.at[5])
    cp_w3 = pltpu.make_async_copy(w3_hbm, w3_s, sems.at[6])
    cp_w4 = pltpu.make_async_copy(w4_hbm, w4_s, sems.at[7])
    cp_out = pltpu.make_async_copy(out_s, out_hbm, sems.at[8])

    def kpiece(sl, rs):
        acc = None
        for t in range(NC):
            o = _dot(ckv_s[t, rs, :], wuk_s[sl, t * 128:(t + 1) * 128, :])
            acc = o if acc is None else acc + o
        kT_s[:, rs] = acc.astype(bf16).T

    def vpiece(sl, rs):
        acc = None
        for t in range(NC):
            o = _dot(ckv_s[t, rs, :], wuv_s[sl, t * 128:(t + 1) * 128, :])
            acc = o if acc is None else acc + o
        v_s[rs, :] = acc.astype(bf16)

    def qpiece(sl, rs):
        acc = None
        for t in range(NP):
            o = _dot(hmod_s[t, rs, :], wq_s[sl, t * 128:(t + 1) * 128, :])
            acc = o if acc is None else acc + o
        q_s[rs, :] = (acc * QSCALE).astype(bf16)

    @pl.when(h == 0)
    def _prologue():
        for cp in cp_ckv:
            cp.start()
        for cp in pcopies(0, 0):
            cp.start()
        cp_wmod.start(); cp_x.start()
        for cp in pcopies(1, 1):
            cp.start()
        wocopy(0, 0).start()
        cp_w1.start(); cp_w2.start(); cp_w3.start(); cp_w4.start()
        x2_s[...] = jnp.zeros((S, M), f32)
        cp_wmod.wait()
        c = c_ref[...].astype(f32)
        sc = c * (1.0 / (1.0 + jnp.exp(-c)))
        sc8 = jnp.broadcast_to(sc, (16, M)).astype(bf16)
        mod = _dot(sc8, wmod_s[...])
        mod_s[...] = mod[0:8, :]
        cp_x.wait()
        sa = mod_s[0:1, 0:M]
        ca = mod_s[0:1, M:2 * M]

        def ln_body(i, carry):
            r = pl.ds(pl.multiple_of(i * 256, 256), 256)
            xb = x_s[r, :].astype(f32)
            hb = (_ln(xb) * (1.0 + ca) + sa).astype(bf16)
            for t in range(NP):
                hmod_s[t, r, :] = hb[:, t * 128:(t + 1) * 128]
            return carry
        lax.fori_loop(0, S // 256, ln_body, 0)
        for cp in cp_ckv:
            cp.wait()
        for cp in pcopies(0, 0):
            cp.wait()

        def proj_body(i, carry):
            rs = pl.ds(pl.multiple_of(i * 512, 512), 512)
            kpiece(0, rs); vpiece(0, rs); qpiece(0, rs)
            return carry
        lax.fori_loop(0, S // 512, proj_body, 0)

    nslot = 1 - slot
    for cp in pcopies(jnp.minimum(h + 1, H - 1), nslot):
        cp.wait()
    wocopy(h, slot).wait()

    @pl.when(h < H - 1)
    def _():
        for cp in pcopies(jnp.minimum(h + 2, H - 1), slot):
            cp.start()
        wocopy(h + 1, nslot).start()

    row = lax.broadcasted_iota(jnp.int32, (128, 128), 0)
    col = lax.broadcasted_iota(jnp.int32, (128, 128), 1)
    causal = col <= row
    nq = S // BQ

    def qk_tiles(i, c0, cw):
        r0 = i * BQ
        q_i = q_s[r0:r0 + BQ, :]
        s = _dot(q_i, kT_s[:, c0:c0 + cw])
        res = []
        for t in range(cw // 128):
            cc = c0 + t * 128
            st = s[:, t * 128:(t + 1) * 128]
            if cc + 128 > r0:
                parts = []
                for rr in range(BQ // 128):
                    rbase = r0 + rr * 128
                    if cc == rbase:
                        parts.append(jnp.where(causal, st[rr * 128:(rr + 1) * 128], NEG))
                    elif cc < rbase:
                        parts.append(st[rr * 128:(rr + 1) * 128])
                    else:
                        parts.append(jnp.full((128, 128), NEG, f32))
                st = parts[0] if len(parts) == 1 else jnp.concatenate(parts, axis=0)
            res.append(st)
        return res

    def chunks(i, cwmax):
        L = (i + 1) * BQ
        return [(c0, min(cwmax, L - c0)) for c0 in range(0, L, cwmax)]

    def rowmax(tiles):
        m = tiles[0]
        for st in tiles[1:]:
            m = jnp.maximum(m, st)
        m = jnp.max(m, axis=-1, keepdims=True)
        return jnp.broadcast_to(m, (BQ, 128))

    order = list(range(nq - 1, -1, -1))
    cur = []
    for (c0, cw) in chunks(order[0], KC):
        cur += qk_tiles(order[0], c0, cw)
    mb = rowmax(cur)
    pending = []
    dead_lo = S
    for oi, i in enumerate(order):
        inext = order[oi + 1] if oi + 1 < nq else None
        nxt_chunks = chunks(inext, KC) if inext is not None else []
        nxt = []
        l = None
        acc = None
        ci = 0
        pv_chunks = chunks(i, PVC)
        npv = len(pv_chunks)
        for pi, (c0, cw) in enumerate(pv_chunks):
            while ci < len(nxt_chunks) and ci * npv < (pi + 1) * len(nxt_chunks) and PIPE:
                nxt += qk_tiles(inext, *nxt_chunks[ci])
                ci += 1
            ps = [jnp.exp2(cur[t] - mb) for t in range(c0 // 128, (c0 + cw) // 128)]
            psum = ps[0]
            for p in ps[1:]:
                psum = psum + p
            l = psum if l is None else l + psum
            pj = ps[0] if len(ps) == 1 else jnp.concatenate(ps, axis=1)
            o = _dot(pj.astype(bf16), v_s[c0:c0 + cw, :])
            acc = o if acc is None else acc + o
            nemit = -(-len(pending) // (npv - pi))
            for _ in range(nemit):
                pending.pop(0)()
        while ci < len(nxt_chunks):
            nxt += qk_tiles(inext, *nxt_chunks[ci])
            ci += 1
        l = jnp.sum(l, axis=-1, keepdims=True)
        r = pl.reciprocal(l, approx=True)
        r = r * (2.0 - l * r)
        ctx = (acc * r).astype(bf16)
        rs = slice(i * BQ, (i + 1) * BQ)
        x2_s[rs, :] = x2_s[rs, :] + _dot(ctx, wo_s[slot])
        if (i * BQ) % PR == 0:
            prs = slice(i * BQ, i * BQ + PR)
            pending += [lambda prs=prs: kpiece(nslot, prs), lambda prs=prs: vpiece(nslot, prs),
                        lambda prs=prs: qpiece(nslot, prs)]
        if not PDELAY:
            while pending:
                pending.pop(0)()
        if nxt:
            cur = nxt
            mb = rowmax(cur)
    while pending:
        pending.pop(0)()

    @pl.when(h == H - 1)
    def _epilogue():
        cp_w1.wait(); cp_w2.wait(); cp_w3.wait(); cp_w4.wait()
        ga = mod_s[0:1, 2 * M:3 * M]
        sb = mod_s[0:1, 3 * M:4 * M]
        cb = mod_s[0:1, 4 * M:5 * M]
        gb = mod_s[0:1, 5 * M:6 * M]
        h1_s[0:8, :] = jnp.zeros((8, M), f32)
        h1_s[S + 8:S + 16, :] = jnp.zeros((8, M), f32)

        def pass1(i, carry):
            r0 = pl.multiple_of(i * RB, RB)
            r = pl.ds(r0, RB)
            x2 = x_s[r, :].astype(f32) + ga * x2_s[r, :]
            x2_s[r, :] = x2
            hb = _ln(x2) * (1.0 + cb) + sb
            h_s[r, :] = hb
            g = _gelu(_dot(_ln(hb).astype(bf16), w1_s[...]))
            h1_s[pl.ds(r0 + 8, RB), :] = g
            return carry
        lax.fori_loop(0, S // RB, pass1, 0)

        lane = lax.broadcasted_iota(jnp.int32, (RB, 128), 1)

        def pass2(i, carry):
            r0 = pl.multiple_of(i * RB, RB)
            r = pl.ds(r0, RB)
            win = h1_s[pl.ds(r0, RB + 16), :]

            def sh(off, t):
                return win[8 + off:8 + off + RB, t * 128:(t + 1) * 128]
            t0 = sh(-1, 0)
            t1 = jnp.where(lane < 32, sh(-1, 1), sh(1, 1))
            t2 = jnp.where(lane < 64, sh(1, 2), sh(-2, 2))
            t3 = jnp.where(lane < 96, sh(-2, 3), sh(2, 3))
            t4 = sh(2, 4)
            g = jnp.concatenate([t0, t1, t2, t3, t4], axis=1).astype(bf16)
            x1 = h_s[r, :] + _dot(g, w2_s[...])
            u = _gelu(_dot(_ln(x1).astype(bf16), w3_s[...])).astype(bf16)
            h2 = _dot(u, w4_s[...])
            out = x2_s[r, :] + gb * (x1 + h2)
            out_s[r, :] = out.astype(bf16)
            return carry
        lax.fori_loop(0, S // RB, pass2, 0)
        cp_out.start()
        cp_out.wait()


@jax.jit
def pallas_adaLN_cond__compressed_kv_cla__mixer_s_mlp__prompt_kernel(
        A_x, A_c_kv, A_w_q, A_w_uk, A_w_uv, A_w_o, B_x, B_w1, B_w2, B_w3, B_w4, c, w_mod):
    x = A_x.reshape(S, M)
    ckv = A_c_kv.reshape(S, DC)
    wq = A_w_q.reshape(M, H * D)
    wuk = A_w_uk.reshape(DC, H * D)
    wuv = A_w_uv.reshape(DC, H * D)
    wo = A_w_o.reshape(H * D, M)
    hbm = pl.BlockSpec(memory_space=pltpu.HBM)
    out = pl.pallas_call(
        _kernel,
        grid=(H,),
        in_specs=[hbm, hbm, hbm, hbm, hbm, hbm, hbm, hbm, hbm, hbm,
                  pl.BlockSpec((1, M), lambda h: (0, 0)),
                  hbm],
        out_specs=hbm,
        out_shape=jax.ShapeDtypeStruct((S, M), bf16),
        scratch_shapes=[
            pltpu.VMEM((S, M), bf16),
            pltpu.VMEM((NC, S, 128), bf16),
            pltpu.VMEM((NP, S, 128), bf16),
            pltpu.VMEM((M, 6 * M), bf16),
            pltpu.VMEM((8, 6 * M), f32),
            pltpu.VMEM((2, D, M), bf16),
            pltpu.VMEM((M, M), bf16),
            pltpu.VMEM((M, M), bf16),
            pltpu.VMEM((M, F), bf16),
            pltpu.VMEM((F, M), bf16),
            pltpu.VMEM((2, M, D), bf16),
            pltpu.VMEM((2, DC, D), bf16),
            pltpu.VMEM((2, DC, D), bf16),
            pltpu.VMEM((S, D), bf16), pltpu.VMEM((D, S), bf16), pltpu.VMEM((S, D), bf16),
            pltpu.VMEM((S, M), f32),
            pltpu.VMEM((S + 16, M), f32),
            pltpu.VMEM((S, M), f32),
            pltpu.VMEM((S, M), bf16),
            pltpu.SemaphoreType.DMA((16,)),
            pltpu.SemaphoreType.DMA((4, 2)),
        ],
        compiler_params=pltpu.CompilerParams(
            dimension_semantics=("arbitrary",),
            vmem_limit_bytes=110 * 1024 * 1024,
            flags=FLAGS,
        ),
    )(x, ckv, wq, wuk, wuv, wo, B_w1, B_w2, B_w3, B_w4, c, w_mod)
    return out.reshape(1, S, M)
```

```python
import os
import numpy as np
import jax
import jax.numpy as jnp
from jax import lax
import jax.experimental.pallas as pl
import jax.experimental.pallas.tpu as pltpu

FP = 1792
S = 2048; M = 640; H = 32; D = 128; DC = 512; F = 1728
BQ = int(os.environ.get("BQ", 128))
KC = int(os.environ.get("KC", 1024))
PVC = int(os.environ.get("PVC", 1024))
PR = int(os.environ.get("PR", 128))
PIPE = int(os.environ.get("PIPE", 1))
PDELAY = int(os.environ.get("PDELAY", 1))
ORD = int(os.environ.get("ORD", 1))
EARLY = int(os.environ.get("EARLY", 0))
LSUM = int(os.environ.get("LSUM", 0))
THR = int(os.environ.get("THR", 1))
THRX = int(os.environ.get("THRX", 0))
RB = int(os.environ.get("RB", 256))
FLAGS = {k: True for k in os.environ.get("KFLAGS", "").split(",") if k} or None
LOG2E = 1.4426950408889634
QSCALE = float(D ** -0.5) * LOG2E
f32 = jnp.float32; bf16 = jnp.bfloat16
NEG = -1e30
NP = M // 128
NC = DC // 128


def _ln(x):
    m = jnp.mean(x, axis=-1, keepdims=True)
    xc = x - m
    v = jnp.mean(xc * xc, axis=-1, keepdims=True)
    return xc * lax.rsqrt(v + 1e-5)


def _gelu(x):
    c0 = float(np.sqrt(2.0 / np.pi))
    u = c0 * (x + 0.044715 * (x * x * x))
    return 0.5 * x * (1.0 + jnp.tanh(u))


def _dot(a, b):
    return jnp.dot(a, b, preferred_element_type=f32)


def _kernel(x_hbm, ckv_hbm, wq_hbm, wuk_hbm, wuv_hbm, wo_hbm, w1_hbm, w2_hbm, w3_hbm, w4_hbm, c_ref, wmod_hbm,
            out_hbm,
            x_s, ckv_s, hmod_s, wmod_s, mod_s, wo_s, w1_s, w2_s, w3_s, w4_s,
            wq_s, wuk_s, wuv_s, rq_s, ruk_s, ruv_s, w3t_s,
            q_s, kT_s, v_s, h_s, h1_s, x2_s, out_s, sems, wsems):
    u32 = jnp.uint32
    wq_pairs = wq_hbm.bitcast(u32)
    wuk_pairs = wuk_hbm.bitcast(u32)
    wuv_pairs = wuv_hbm.bitcast(u32)

    def pcopies(hh, sl):
        j = hh // 2
        return [pltpu.make_async_copy(wq_pairs.at[:, j, :], rq_s.at[sl], wsems.at[0, sl]),
                pltpu.make_async_copy(wuk_pairs.at[:, j, :], ruk_s.at[sl], wsems.at[1, sl]),
                pltpu.make_async_copy(wuv_pairs.at[:, j, :], ruv_s.at[sl], wsems.at[2, sl])]

    def unpack_weights(hh, sl):
        sh = jnp.asarray(16 * (1 - hh % 2)).astype(u32)
        for raw, dst in ((rq_s, wq_s), (ruk_s, wuk_s), (ruv_s, wuv_s)):
            bits = (raw[sl] << sh) & jnp.uint32(0xFFFF0000)
            dst[...] = pltpu.bitcast(bits, f32).astype(bf16)

    def wocopy(hh, sl):
        return pltpu.make_async_copy(wo_hbm.at[pl.ds(pl.multiple_of(hh * D, D), D), :], wo_s.at[sl], wsems.at[3, sl])

    cp_x = pltpu.make_async_copy(x_hbm, x_s, sems.at[0])
    cp_ckv = [pltpu.make_async_copy(ckv_hbm.at[:, t * 128:(t + 1) * 128], ckv_s.at[t], sems.at[9 + t]) for t in range(NC)]
    cp_wmod0 = pltpu.make_async_copy(wmod_hbm.at[:, 0:2 * M], wmod_s.at[:, 0:2 * M], sems.at[2])
    cp_wmod1 = pltpu.make_async_copy(wmod_hbm.at[:, 2 * M:6 * M], wmod_s.at[:, 2 * M:6 * M], sems.at[3])
    cp_w1 = pltpu.make_async_copy(w1_hbm, w1_s, sems.at[4])
    cp_w2 = pltpu.make_async_copy(w2_hbm, w2_s, sems.at[5])
    cp_w3 = pltpu.make_async_copy(w3_hbm, w3t_s, sems.at[6])
    cp_w4 = pltpu.make_async_copy(w4_hbm, w4_s.at[0:F, :], sems.at[7])
    cp_out = pltpu.make_async_copy(out_s, out_hbm, sems.at[8])

    def kpiece(sl, rs):
        acc = None
        for t in range(NC):
            o = _dot(ckv_s[t, rs, :], wuk_s[t * 128:(t + 1) * 128, :])
            acc = o if acc is None else acc + o
        kT_s[:, rs] = acc.astype(bf16).T

    def vpiece(sl, rs):
        acc = None
        for t in range(NC):
            o = _dot(ckv_s[t, rs, :], wuv_s[t * 128:(t + 1) * 128, :])
            acc = o if acc is None else acc + o
        v_s[rs, :] = acc.astype(bf16)

    def qpiece(sl, rs):
        acc = None
        for t in range(NP):
            o = _dot(hmod_s[t, rs, :], wq_s[t * 128:(t + 1) * 128, :])
            acc = o if acc is None else acc + o
        q_s[rs, :] = (acc * QSCALE).astype(bf16)

    def prologue():
        for cp in cp_ckv:
            cp.start()
        for cp in pcopies(0, 0):
            cp.start()
        cp_wmod0.start(); cp_x.start()
        for cp in pcopies(1, 1):
            cp.start()
        wocopy(0, 0).start()
        cp_wmod1.start()
        cp_w1.start(); cp_w2.start(); cp_w3.start(); cp_w4.start()
        x2_s[...] = jnp.zeros((S, M), f32)
        h1_s[0:8, :] = jnp.zeros((8, M), f32)
        h1_s[S + 8:S + 16, :] = jnp.zeros((8, M), f32)
        w3_s[:, F:FP] = jnp.zeros((M, FP - F), bf16)
        w4_s[F:FP, :] = jnp.zeros((FP - F, M), bf16)
        for cp in cp_ckv:
            cp.wait()
        for cp in pcopies(0, 0):
            cp.wait()
        unpack_weights(0, 0)

        def kv_body(i, carry):
            rs = pl.ds(pl.multiple_of(i * 512, 512), 512)
            kpiece(0, rs); vpiece(0, rs)
            return carry
        lax.fori_loop(0, S // 512, kv_body, 0)

        cp_wmod0.wait()
        c = c_ref[...].astype(f32)
        sc = c * (1.0 / (1.0 + jnp.exp(-c)))
        sc8 = jnp.broadcast_to(sc, (16, M)).astype(bf16)
        mod_s[:, 0:2 * M] = _dot(sc8, wmod_s[:, 0:2 * M])[0:8, :]
        cp_x.wait()
        sa = mod_s[0:1, 0:M]
        ca = mod_s[0:1, M:2 * M]

        def ln_body(i, carry):
            r = pl.ds(pl.multiple_of(i * 256, 256), 256)
            xb = x_s[r, :].astype(f32)
            hb = (_ln(xb) * (1.0 + ca) + sa).astype(bf16)
            for t in range(NP):
                hmod_s[t, r, :] = hb[:, t * 128:(t + 1) * 128]
            qpiece(0, r)
            return carry
        lax.fori_loop(0, S // 256, ln_body, 0)
        return sc8

    sc8 = prologue()

    def head_body(h, carry):
        slot = h % 2
        nslot = 1 - slot
        for cp in pcopies(jnp.minimum(h + 1, H - 1), nslot):
            cp.wait()
        wocopy(h, slot).wait()

        unpack_weights(jnp.minimum(h + 1, H - 1), nslot)

        @pl.when(h < H - 1)
        def _():
            for cp in pcopies(jnp.minimum(h + 2, H - 1), slot):
                cp.start()
            wocopy(h + 1, nslot).start()

        row = lax.broadcasted_iota(jnp.int32, (128, 128), 0)
        col = lax.broadcasted_iota(jnp.int32, (128, 128), 1)
        causal = col <= row
        nq = S // BQ

        def qk_tiles(i, c0, cw):
            r0 = i * BQ
            q_i = q_s[r0:r0 + BQ, :]
            s = _dot(q_i, kT_s[:, c0:c0 + cw])
            res = []
            for t in range(cw // 128):
                cc = c0 + t * 128
                st = s[:, t * 128:(t + 1) * 128]
                if cc + 128 > r0:
                    parts = []
                    for rr in range(BQ // 128):
                        rbase = r0 + rr * 128
                        if cc == rbase:
                            parts.append(jnp.where(causal, st[rr * 128:(rr + 1) * 128], NEG))
                        elif cc < rbase:
                            parts.append(st[rr * 128:(rr + 1) * 128])
                        else:
                            parts.append(jnp.full((128, 128), NEG, f32))
                    st = parts[0] if len(parts) == 1 else jnp.concatenate(parts, axis=0)
                res.append(st)
            return res

        def chunks(i, cwmax):
            L = (i + 1) * BQ
            return [(c0, min(cwmax, L - c0)) for c0 in range(0, L, cwmax)]

        def rowmax(tiles):
            m = tiles[0]
            for st in tiles[1:]:
                m = jnp.maximum(m, st)
            m = jnp.max(m, axis=-1, keepdims=True)
            return jnp.broadcast_to(m, (BQ, 128))

        order = list(range(nq - 1, -1, -1))
        pending = []

        def add_kq(i):
            if (i * BQ) % PR == 0:
                prs = slice(i * BQ, i * BQ + PR)
                pending.append(lambda: kpiece(nslot, prs))
                pending.append(lambda: qpiece(nslot, prs))

        def add_v(i):
            if (i * BQ) % PR == 0:
                prs = slice(i * BQ, i * BQ + PR)
                pending.append(lambda: vpiece(nslot, prs))

        olds = []
        cur = []
        for (c0, cw) in chunks(order[0], KC):
            cur += qk_tiles(order[0], c0, cw)
        mb = rowmax(cur)
        if EARLY:
            add_kq(order[0])
        for oi, i in enumerate(order):
            inext = order[oi + 1] if oi + 1 < nq else None
            nxt_chunks = chunks(inext, KC) if inext is not None else []
            nxt = []
            l = None
            acc = None
            ci = 0
            pv_chunks = chunks(i, PVC)
            npv = len(pv_chunks)
            if not THRX:
                olds = []
            for pi, (c0, cw) in enumerate(pv_chunks):
                def emit_qk():
                    nonlocal ci, nxt
                    while ci < len(nxt_chunks) and ci * npv < (pi + 1) * len(nxt_chunks):
                        nxt += qk_tiles(inext, *nxt_chunks[ci])
                        ci += 1
                if ORD == 0:
                    emit_qk()
                mbc = mb
                if THR and len(olds) >= THR:
                    mbc = mb + olds[-THR] * 0.0
                ps = [jnp.exp2(cur[t] - mbc) for t in range(c0 // 128, (c0 + cw) // 128)]
                pj = ps[0] if len(ps) == 1 else jnp.concatenate(ps, axis=1)
                pj = pj.astype(bf16)
                if LSUM == 1:
                    pf = pj.astype(f32)
                    ps = [pf[:, t * 128:(t + 1) * 128] for t in range(cw // 128)]
                if LSUM == 2:
                    for p in ps:
                        l = p if l is None else l + p
                else:
                    psum = ps[0]
                    for p in ps[1:]:
                        psum = psum + p
                    l = psum if l is None else l + psum
                o = _dot(pj, v_s[c0:c0 + cw, :])
                olds.append(o)
                acc = o if acc is None else acc + o
                if ORD == 1:
                    emit_qk()
                nemit = -(-len(pending) // (npv - pi))
                for _ in range(nemit):
                    pending.pop(0)()
                if ORD == 2:
                    emit_qk()
            if EARLY and inext is not None:
                add_kq(inext)
            l = jnp.sum(l, axis=-1, keepdims=True)
            r = pl.reciprocal(l, approx=True)
            r = r * (2.0 - l * r)
            ctx = (acc * r).astype(bf16)
            rs = slice(i * BQ, i * BQ + BQ)
            x2_s[rs, :] = x2_s[rs, :] + _dot(ctx, wo_s[slot])
            if not EARLY:
                add_kq(i)
            add_v(i)
            if not PDELAY:
                while pending:
                    pending.pop(0)()
            if nxt:
                cur = nxt
                mb = rowmax(cur)
        while pending:
            pending.pop(0)()

        return carry

    lax.fori_loop(0, H, head_body, 0)

    def epilogue():
        cp_wmod1.wait()
        mod_s[:, 2 * M:6 * M] = _dot(sc8, wmod_s[:, 2 * M:6 * M])[0:8, :]
        cp_w1.wait(); cp_w2.wait(); cp_w3.wait(); cp_w4.wait()
        ga = mod_s[0:1, 2 * M:3 * M]
        sb = mod_s[0:1, 3 * M:4 * M]
        cb = mod_s[0:1, 4 * M:5 * M]
        gb = mod_s[0:1, 5 * M:6 * M]
        for t in range(FP // 128):
            n = min(128, F - t * 128)
            w3_s[:, t * 128:t * 128 + n] = w3t_s[t * 128:t * 128 + n, :].T

        def pass1(i, carry):
            r0 = pl.multiple_of(i * RB, RB)
            r = pl.ds(r0, RB)
            x2 = x_s[r, :].astype(f32) + ga * x2_s[r, :]
            x2_s[r, :] = x2
            hb = _ln(x2) * (1.0 + cb) + sb
            h_s[r, :] = hb
            g = _gelu(_dot(_ln(hb).astype(bf16), w1_s[...]))
            h1_s[pl.ds(r0 + 8, RB), :] = g
            return carry
        lax.fori_loop(0, S // RB, pass1, 0)

        lane = lax.broadcasted_iota(jnp.int32, (RB, 128), 1)

        def pass2(i, carry):
            r0 = pl.multiple_of(i * RB, RB)
            r = pl.ds(r0, RB)
            win = h1_s[pl.ds(r0, RB + 16), :]

            def sh(off, t):
                return win[8 + off:8 + off + RB, t * 128:(t + 1) * 128]
            t0 = sh(-1, 0)
            t1 = jnp.where(lane < 32, sh(-1, 1), sh(1, 1))
            t2 = jnp.where(lane < 64, sh(1, 2), sh(-2, 2))
            t3 = jnp.where(lane < 96, sh(-2, 3), sh(2, 3))
            t4 = sh(2, 4)
            g = jnp.concatenate([t0, t1, t2, t3, t4], axis=1).astype(bf16)
            x1 = h_s[r, :] + _dot(g, w2_s[...])
            u = _gelu(_dot(_ln(x1).astype(bf16), w3_s[...])).astype(bf16)
            h2 = _dot(u, w4_s[...])
            out = x2_s[r, :] + gb * (x1 + h2)
            out_s[r, :] = out.astype(bf16)
            return carry
        lax.fori_loop(0, S // RB, pass2, 0)
        cp_out.start()
        cp_out.wait()

    epilogue()


@jax.jit
def pallas_adaLN_cond__compressed_kv_cla__mixer_s_mlp__prompt_kernel(
        A_x, A_c_kv, A_w_q, A_w_uk, A_w_uv, A_w_o, B_x, B_w1, B_w2, B_w3, B_w4, c, w_mod):
    x = A_x.reshape(S, M)
    ckv = A_c_kv.reshape(S, DC)
    wq, wuk, wuv = A_w_q, A_w_uk, A_w_uv
    wo = A_w_o.reshape(H * D, M)
    hbm = pl.BlockSpec(memory_space=pltpu.HBM)
    out = pl.pallas_call(
        _kernel,
        grid=(1,),
        in_specs=[hbm, hbm, hbm, hbm, hbm, hbm, hbm, hbm, hbm, hbm,
                  pl.BlockSpec((1, M), lambda h: (0, 0)),
                  hbm],
        out_specs=hbm,
        out_shape=jax.ShapeDtypeStruct((S, M), bf16),
        scratch_shapes=[
            pltpu.VMEM((S, M), bf16),
            pltpu.VMEM((NC, S, 128), bf16),
            pltpu.VMEM((NP, S, 128), bf16),
            pltpu.VMEM((M, 6 * M), bf16),
            pltpu.VMEM((8, 6 * M), f32),
            pltpu.VMEM((2, D, M), bf16),
            pltpu.VMEM((M, M), bf16),
            pltpu.VMEM((M, M), bf16),
            pltpu.VMEM((M, FP), bf16),
            pltpu.VMEM((FP, M), bf16),
            pltpu.VMEM((M, D), bf16),
            pltpu.VMEM((DC, D), bf16),
            pltpu.VMEM((DC, D), bf16),
            pltpu.VMEM((2, M, D), jnp.uint32),
            pltpu.VMEM((2, DC, D), jnp.uint32),
            pltpu.VMEM((2, DC, D), jnp.uint32),
            pltpu.VMEM((F, M), bf16),
            pltpu.VMEM((S, D), bf16), pltpu.VMEM((D, S), bf16), pltpu.VMEM((S, D), bf16),
            pltpu.VMEM((S, M), f32),
            pltpu.VMEM((S + 16, M), f32),
            pltpu.VMEM((S, M), f32),
            pltpu.VMEM((S, M), bf16),
            pltpu.SemaphoreType.DMA((16,)),
            pltpu.SemaphoreType.DMA((4, 2)),
        ],
        compiler_params=pltpu.CompilerParams(
            dimension_semantics=("arbitrary",),
            vmem_limit_bytes=110 * 1024 * 1024,
            flags=FLAGS,
        ),
    )(x, ckv, wq, wuk, wuv, wo, B_w1, B_w2, B_w3.T, B_w4, c, w_mod)
    return out.reshape(1, S, M)
```

```python
import os
import numpy as np
import jax
import jax.numpy as jnp
from jax import lax
import jax.experimental.pallas as pl
import jax.experimental.pallas.tpu as pltpu

FP = 1792
PB = 256
S = 2048; M = 640; H = 32; D = 128; DC = 512; F = 1728
BQ = int(os.environ.get("BQ", 128))
KC = int(os.environ.get("KC", 1024))
PVC = int(os.environ.get("PVC", 1024))
PR = int(os.environ.get("PR", 128))
OPD = int(os.environ.get('OPD', 0))
OPD_SPREAD = int(os.environ.get('OPD_SPREAD', 3))
OPD_N = int(os.environ.get('OPD_N', 6))
EPI = int(os.environ.get('EPI', 0))
LOOK = int(os.environ.get('LOOK', 2))
PIPE = int(os.environ.get("PIPE", 1))
PDELAY = int(os.environ.get("PDELAY", 1))
ORD = int(os.environ.get("ORD", 1))
EARLY = int(os.environ.get("EARLY", 0))
LSUM = int(os.environ.get("LSUM", 0))
THR = int(os.environ.get("THR", 1))
THRX = int(os.environ.get("THRX", 0))
RB = int(os.environ.get("RB", 256))
FLAGS = {k: True for k in os.environ.get("KFLAGS", "").split(",") if k} or None
LOG2E = 1.4426950408889634
QSCALE = float(D ** -0.5) * LOG2E
f32 = jnp.float32; bf16 = jnp.bfloat16
NEG = -1e30
NP = M // 128
NC = DC // 128


def _ln(x):
    m = jnp.mean(x, axis=-1, keepdims=True)
    xc = x - m
    v = jnp.mean(xc * xc, axis=-1, keepdims=True)
    return xc * lax.rsqrt(v + 1e-5)


def _gelu(x):
    c0 = float(np.sqrt(2.0 / np.pi))
    u = c0 * (x + 0.044715 * (x * x * x))
    return 0.5 * x * (1.0 + jnp.tanh(u))


def _dot(a, b):
    return jnp.dot(a, b, preferred_element_type=f32)


def _kernel(x_hbm, ckv_hbm, wq_hbm, wuk_hbm, wuv_hbm, wo_hbm, w1_hbm, w2_hbm, w3_hbm, w4_hbm, c_ref, wmod_hbm,
            out_hbm,
            x_s, ckv_s, hmod_s, wmod_s, mod_s, wo_s, w1_s, w2_s, w3_s, w4_s,
            wq_s, wuk_s, wuv_s, rq_s, ruk_s, ruv_s, w3t_s,
            q_s, kT_s, v_s, ctx_s, h_s, h1_s, acc_s, x2_s, out_s, sems, wsems, isems):
    u32 = jnp.uint32
    wq_pairs = wq_hbm.bitcast(u32)
    wuk_pairs = wuk_hbm.bitcast(u32)
    wuv_pairs = wuv_hbm.bitcast(u32)

    def pcopies(hh, sl):
        j = hh // 2
        return [pltpu.make_async_copy(wq_pairs.at[:, j, :], rq_s.at[sl], wsems.at[0, sl]),
                pltpu.make_async_copy(wuk_pairs.at[:, j, :], ruk_s.at[sl], wsems.at[1, sl]),
                pltpu.make_async_copy(wuv_pairs.at[:, j, :], ruv_s.at[sl], wsems.at[2, sl])]

    def unpack_weights(hh, sl):
        sh = jnp.asarray(16 * (1 - hh % 2)).astype(u32)
        for raw, dst in ((rq_s, wq_s), (ruk_s, wuk_s), (ruv_s, wuv_s)):
            bits = (raw[sl] << sh) & jnp.uint32(0xFFFF0000)
            dst[...] = pltpu.bitcast(bits, f32).astype(bf16)

    def wocopy(hh, sl):
        return pltpu.make_async_copy(wo_hbm.at[pl.ds(pl.multiple_of(hh * D, D), D), :], wo_s.at[sl], wsems.at[3, sl])

    def in_copies(i):
        r = pl.ds(pl.multiple_of(i * PB, PB), PB)
        return [pltpu.make_async_copy(x_hbm.at[r, :], x_s.at[r, :], isems.at[0, i]),
                pltpu.make_async_copy(ckv_hbm.at[r, :], ckv_s.at[r, :], isems.at[1, i])]

    cp_wmod0 = pltpu.make_async_copy(wmod_hbm.at[:, 0:2 * M], wmod_s.at[:, 0:2 * M], sems.at[2])
    cp_wmod1 = pltpu.make_async_copy(wmod_hbm.at[:, 2 * M:6 * M], wmod_s.at[:, 2 * M:6 * M], sems.at[3])
    cp_w1 = pltpu.make_async_copy(w1_hbm, w1_s, sems.at[4])
    cp_w2 = pltpu.make_async_copy(w2_hbm, w2_s, sems.at[5])
    cp_w3 = pltpu.make_async_copy(w3_hbm, w3t_s, sems.at[6])
    cp_w4 = pltpu.make_async_copy(w4_hbm, w4_s.at[0:F, :], sems.at[7])
    cp_out = pltpu.make_async_copy(out_s, out_hbm, sems.at[8])

    def kpiece(sl, rs):
        acc = None
        for t in range(NC):
            o = _dot(ckv_s[rs, t * 128:(t + 1) * 128], wuk_s[t * 128:(t + 1) * 128, :])
            acc = o if acc is None else acc + o
        kT_s[:, rs] = acc.astype(bf16).T

    def vpiece(sl, rs):
        acc = None
        for t in range(NC):
            o = _dot(ckv_s[rs, t * 128:(t + 1) * 128], wuv_s[t * 128:(t + 1) * 128, :])
            acc = o if acc is None else acc + o
        v_s[rs, :] = acc.astype(bf16)

    def qpiece(sl, rs):
        acc = None
        for t in range(NP):
            o = _dot(hmod_s[rs, t * 128:(t + 1) * 128], wq_s[t * 128:(t + 1) * 128, :])
            acc = o if acc is None else acc + o
        q_s[rs, :] = (acc * QSCALE).astype(bf16)

    def prologue():
        cp_wmod0.start()
        for cp in pcopies(0, 0):
            cp.start()
        for i in range(LOOK):
            for cp in in_copies(i):
                cp.start()
        acc_s[...] = jnp.zeros((S, M), f32)
        h1_s[0:8, :] = jnp.zeros((8, M), f32)
        h1_s[S + 8:S + 16, :] = jnp.zeros((8, M), f32)
        w3_s[:, F:FP] = jnp.zeros((M, FP - F), bf16)
        w4_s[F:FP, :] = jnp.zeros((FP - F, M), bf16)

        c = c_ref[...].astype(f32)
        sc = c * (1.0 / (1.0 + jnp.exp(-c)))
        sc8 = jnp.broadcast_to(sc, (16, M)).astype(bf16)
        cp_wmod0.wait()
        mod_s[:, 0:2 * M] = _dot(sc8, wmod_s[:, 0:2 * M])[0:8, :]
        sa = mod_s[0:1, 0:M]
        ca = mod_s[0:1, M:2 * M]
        for cp in pcopies(0, 0):
            cp.wait()
        unpack_weights(0, 0)

        def first_body(i, carry):
            r = pl.ds(pl.multiple_of(i * PB, PB), PB)
            for cp in in_copies(i):
                cp.wait()

            @pl.when(i + LOOK < S // PB)
            def _():
                for cp in in_copies(i + LOOK):
                    cp.start()

            @pl.when(i + LOOK == S // PB)
            def _():
                for cp in pcopies(1, 1):
                    cp.start()
                wocopy(0, 0).start()
            xb = x_s[r, :].astype(f32)
            hmod_s[r, :] = (_ln(xb) * (1.0 + ca) + sa).astype(bf16)
            kpiece(0, r); vpiece(0, r); qpiece(0, r)
            return carry
        lax.fori_loop(0, S // PB, first_body, 0)
        cp_wmod1.start()
        cp_w1.start(); cp_w2.start(); cp_w3.start(); cp_w4.start()
        return sc8

    sc8 = prologue()

    def head_body(h, carry):
        slot = h % 2
        nslot = 1 - slot
        for cp in pcopies(jnp.minimum(h + 1, H - 1), nslot):
            cp.wait()
        wocopy(jnp.maximum(h - OPD, 0), slot).wait()
        for cp in pcopies(jnp.minimum(h + 2, H - 1), slot):
            cp.start()
        wocopy(jnp.minimum(h + 1 - OPD, H - 1), nslot).start()
        unpack_weights(jnp.minimum(h + 1, H - 1), nslot)

        row = lax.broadcasted_iota(jnp.int32, (128, 128), 0)
        col = lax.broadcasted_iota(jnp.int32, (128, 128), 1)
        causal = col <= row
        nq = S // BQ

        def qk_tiles(i, c0, cw):
            r0 = i * BQ
            q_i = q_s[r0:r0 + BQ, :]
            s = _dot(q_i, kT_s[:, c0:c0 + cw])
            res = []
            for t in range(cw // 128):
                cc = c0 + t * 128
                st = s[:, t * 128:(t + 1) * 128]
                if cc + 128 > r0:
                    parts = []
                    for rr in range(BQ // 128):
                        rbase = r0 + rr * 128
                        if cc == rbase:
                            parts.append(jnp.where(causal, st[rr * 128:(rr + 1) * 128], NEG))
                        elif cc < rbase:
                            parts.append(st[rr * 128:(rr + 1) * 128])
                        else:
                            parts.append(jnp.full((128, 128), NEG, f32))
                    st = parts[0] if len(parts) == 1 else jnp.concatenate(parts, axis=0)
                res.append(st)
            return res

        def chunks(i, cwmax):
            L = (i + 1) * BQ
            return [(c0, min(cwmax, L - c0)) for c0 in range(0, L, cwmax)]

        def rowmax(tiles):
            m = tiles[0]
            for st in tiles[1:]:
                m = jnp.maximum(m, st)
            m = jnp.max(m, axis=-1, keepdims=True)
            return jnp.broadcast_to(m, (BQ, 128))

        order = list(range(nq - 1, -1, -1))
        pending = []

        def add_kq(i):
            if (i * BQ) % PR == 0:
                prs = slice(i * BQ, i * BQ + PR)
                pending.append(lambda: kpiece(nslot, prs))
                pending.append(lambda: qpiece(nslot, prs))

        def add_v(i):
            if (i * BQ) % PR == 0:
                prs = slice(i * BQ, i * BQ + PR)
                pending.append(lambda: vpiece(nslot, prs))

        olds = []
        cur = []
        for (c0, cw) in chunks(order[0], KC):
            cur += qk_tiles(order[0], c0, cw)
        mb = rowmax(cur)
        if EARLY:
            add_kq(order[0])
        if OPD:
            def opiece(rs):
                acc_s[rs, :] = acc_s[rs, :] + _dot(ctx_s[rs, :], wo_s[slot])
            for i_ in order:
                pending.append(lambda rs=slice(i_ * BQ, i_ * BQ + BQ): opiece(rs))
        for oi, i in enumerate(order):
            inext = order[oi + 1] if oi + 1 < nq else None
            nxt_chunks = chunks(inext, KC) if inext is not None else []
            nxt = []
            l = None
            acc = None
            ci = 0
            pv_chunks = chunks(i, PVC)
            npv = len(pv_chunks)
            if not THRX:
                olds = []
            for pi, (c0, cw) in enumerate(pv_chunks):
                def emit_qk():
                    nonlocal ci, nxt
                    while ci < len(nxt_chunks) and ci * npv < (pi + 1) * len(nxt_chunks):
                        nxt += qk_tiles(inext, *nxt_chunks[ci])
                        ci += 1
                if ORD == 0:
                    emit_qk()
                mbc = mb
                if THR and len(olds) >= THR:
                    mbc = mb + olds[-THR] * 0.0
                ps = [jnp.exp2(cur[t] - mbc) for t in range(c0 // 128, (c0 + cw) // 128)]
                pj = ps[0] if len(ps) == 1 else jnp.concatenate(ps, axis=1)
                pj = pj.astype(bf16)
                if LSUM == 1:
                    pf = pj.astype(f32)
                    ps = [pf[:, t * 128:(t + 1) * 128] for t in range(cw // 128)]
                if LSUM == 2:
                    for p in ps:
                        l = p if l is None else l + p
                else:
                    psum = ps[0]
                    for p in ps[1:]:
                        psum = psum + p
                    l = psum if l is None else l + psum
                o = _dot(pj, v_s[c0:c0 + cw, :])
                olds.append(o)
                acc = o if acc is None else acc + o
                if ORD == 1:
                    emit_qk()
                nemit = -(-len(pending) // (npv - pi))
                if OPD and oi < OPD_SPREAD:
                    nemit = min(nemit, -(-OPD_N // npv))
                for _ in range(nemit):
                    pending.pop(0)()
                if ORD == 2:
                    emit_qk()
            if EARLY and inext is not None:
                add_kq(inext)
            l = jnp.sum(l, axis=-1, keepdims=True)
            r = pl.reciprocal(l, approx=True)
            r = r * (2.0 - l * r)
            ctx = (acc * r).astype(bf16)
            rs = slice(i * BQ, i * BQ + BQ)
            if OPD:
                ctx_s[rs, :] = ctx
            else:
                acc_s[rs, :] = acc_s[rs, :] + _dot(ctx, wo_s[slot])
            if not EARLY:
                add_kq(i)
            add_v(i)
            if not PDELAY:
                while pending:
                    pending.pop(0)()
            if nxt:
                cur = nxt
                mb = rowmax(cur)
        while pending:
            pending.pop(0)()

        return carry

    lax.fori_loop(0, H, head_body, 0)
    for cp in pcopies(H - 1, (H - 1) % 2):
        cp.wait()
    wocopy(H - 1, H % 2).wait()

    def epilogue():
        cp_wmod1.wait()
        mod_s[:, 2 * M:6 * M] = _dot(sc8, wmod_s[:, 2 * M:6 * M])[0:8, :]
        cp_w1.wait(); cp_w2.wait(); cp_w3.wait(); cp_w4.wait()
        ga = mod_s[0:1, 2 * M:3 * M]
        sb = mod_s[0:1, 3 * M:4 * M]
        cb = mod_s[0:1, 4 * M:5 * M]
        gb = mod_s[0:1, 5 * M:6 * M]
        for t in range(FP // 128):
            n = min(128, F - t * 128)
            w3_s[:, t * 128:t * 128 + n] = w3t_s[t * 128:t * 128 + n, :].T

        lane = lax.broadcasted_iota(jnp.int32, (RB, 128), 1)

        def pass1(i):
            r0 = pl.multiple_of(i * RB, RB)
            r = pl.ds(r0, RB)
            att = acc_s[r, :]
            if OPD:
                att = att + _dot(ctx_s[r, :], wo_s[H % 2])
            x2 = x_s[r, :].astype(f32) + ga * att
            x2_s[r, :] = x2
            hb = _ln(x2) * (1.0 + cb) + sb
            h_s[r, :] = hb
            g = _gelu(_dot(_ln(hb).astype(bf16), w1_s[...]))
            h1_s[pl.ds(r0 + 8, RB), :] = g

        def pass2(i, mid=None):
            r0 = pl.multiple_of(i * RB, RB)
            r = pl.ds(r0, RB)
            win = h1_s[pl.ds(r0, RB + 16), :]

            def sh(off, t):
                return win[8 + off:8 + off + RB, t * 128:(t + 1) * 128]
            t0 = sh(-1, 0)
            t1 = jnp.where(lane < 32, sh(-1, 1), sh(1, 1))
            t2 = jnp.where(lane < 64, sh(1, 2), sh(-2, 2))
            t3 = jnp.where(lane < 96, sh(-2, 3), sh(2, 3))
            t4 = sh(2, 4)
            g = jnp.concatenate([t0, t1, t2, t3, t4], axis=1).astype(bf16)
            x1 = h_s[r, :] + _dot(g, w2_s[...])
            y = x2_s[r, :] + gb * x1
            ln1 = _ln(x1).astype(bf16)
            if mid is not None:
                mid()
            u = _gelu(_dot(ln1, w3_s[...])).astype(bf16)
            h2 = _dot(u, w4_s[...])
            out_s[r, :] = (y + gb * h2).astype(bf16)
            pltpu.make_async_copy(out_s.at[r, :], out_hbm.at[r, :], sems.at[8]).start()

        NB = S // RB
        if EPI == 0:
            def b1(i, carry):
                pass1(i)
                return carry
            lax.fori_loop(0, NB, b1, 0)

            def b2(i, carry):
                pass2(i)
                return carry
            lax.fori_loop(0, NB, b2, 0)
        else:
            def b1(i, carry):
                pass1(i)
                return carry
            lax.fori_loop(0, 2, b1, 0)

            def b2(i, carry):
                pass2(i, lambda: pass1(jnp.minimum(i + 2, NB - 1)))
                return carry
            lax.fori_loop(0, NB, b2, 0)
        cp_out.wait()

    epilogue()


@jax.jit
def pallas_adaLN_cond__compressed_kv_cla__mixer_s_mlp__prompt_kernel(
        A_x, A_c_kv, A_w_q, A_w_uk, A_w_uv, A_w_o, B_x, B_w1, B_w2, B_w3, B_w4, c, w_mod):
    x = A_x.reshape(S, M)
    ckv = A_c_kv.reshape(S, DC)
    wq, wuk, wuv = A_w_q, A_w_uk, A_w_uv
    wo = A_w_o.reshape(H * D, M)
    hbm = pl.BlockSpec(memory_space=pltpu.HBM)
    out = pl.pallas_call(
        _kernel,
        grid=(1,),
        in_specs=[hbm, hbm, hbm, hbm, hbm, hbm, hbm, hbm, hbm, hbm,
                  pl.BlockSpec((1, M), lambda h: (0, 0)),
                  hbm],
        out_specs=hbm,
        out_shape=jax.ShapeDtypeStruct((S, M), bf16),
        scratch_shapes=[
            pltpu.VMEM((S, M), bf16),
            pltpu.VMEM((S, DC), bf16),
            pltpu.VMEM((S, M), bf16),
            pltpu.VMEM((M, 6 * M), bf16),
            pltpu.VMEM((8, 6 * M), f32),
            pltpu.VMEM((2, D, M), bf16),
            pltpu.VMEM((M, M), bf16),
            pltpu.VMEM((M, M), bf16),
            pltpu.VMEM((M, FP), bf16),
            pltpu.VMEM((FP, M), bf16),
            pltpu.VMEM((M, D), bf16),
            pltpu.VMEM((DC, D), bf16),
            pltpu.VMEM((DC, D), bf16),
            pltpu.VMEM((2, M, D), jnp.uint32),
            pltpu.VMEM((2, DC, D), jnp.uint32),
            pltpu.VMEM((2, DC, D), jnp.uint32),
            pltpu.VMEM((F, M), bf16),
            pltpu.VMEM((S, D), bf16), pltpu.VMEM((D, S), bf16), pltpu.VMEM((S, D), bf16),
            pltpu.VMEM((S, D), bf16),
            pltpu.VMEM((S, M), f32),
            pltpu.VMEM((S + 16, M), f32),
            pltpu.VMEM((S, M), f32),
            pltpu.VMEM((S, M), f32),
            pltpu.VMEM((S, M), bf16),
            pltpu.SemaphoreType.DMA((16,)),
            pltpu.SemaphoreType.DMA((4, 2)),
            pltpu.SemaphoreType.DMA((2, S // PB)),
        ],
        compiler_params=pltpu.CompilerParams(
            dimension_semantics=("arbitrary",),
            vmem_limit_bytes=110 * 1024 * 1024,
            flags=FLAGS,
        ),
    )(x, ckv, wq, wuk, wuv, wo, B_w1, B_w2, B_w3.T, B_w4, c, w_mod)
    return out.reshape(1, S, M)
```

```python
import os
import numpy as np
import jax
import jax.numpy as jnp
from jax import lax
import jax.experimental.pallas as pl
import jax.experimental.pallas.tpu as pltpu

FP = 1792
PB = 256
S = 2048; M = 640; H = 32; D = 128; DC = 512; F = 1728
BQ = int(os.environ.get("BQ", 128))
KC = int(os.environ.get("KC", 1024))
PVC = int(os.environ.get("PVC", 1024))
PR = int(os.environ.get("PR", 128))
OPD = int(os.environ.get('OPD', 0))
OPD_SPREAD = int(os.environ.get('OPD_SPREAD', 3))
OPD_N = int(os.environ.get('OPD_N', 6))
EPI = int(os.environ.get('EPI', 0))
LOOK = int(os.environ.get('LOOK', 2))
W3NT = int(os.environ.get('W3NT', 1))
KNT = int(os.environ.get('KNT', 1))
QDELAY = int(os.environ.get('QDELAY', 8))
QPOS = int(os.environ.get('QPOS', 1))
EORD = int(os.environ.get('EORD', 0))
PORD = int(os.environ.get('PORD', 1))
DPOS = int(os.environ.get('DPOS', 0))
PIPE = int(os.environ.get("PIPE", 1))
PDELAY = int(os.environ.get("PDELAY", 1))
ORD = int(os.environ.get("ORD", 1))
EARLY = int(os.environ.get("EARLY", 0))
LSUM = int(os.environ.get("LSUM", 0))
THR = int(os.environ.get("THR", 1))
THRX = int(os.environ.get("THRX", 0))
RB = int(os.environ.get("RB", 512))
FLAGS = {k: True for k in os.environ.get("KFLAGS", "").split(",") if k} or None
LOG2E = 1.4426950408889634
QSCALE = float(D ** -0.5) * LOG2E
f32 = jnp.float32; bf16 = jnp.bfloat16
NEG = -1e30
NP = M // 128
NC = DC // 128


def _ln(x):
    m = jnp.mean(x, axis=-1, keepdims=True)
    xc = x - m
    v = jnp.mean(xc * xc, axis=-1, keepdims=True)
    return xc * lax.rsqrt(v + 1e-5)


def _gelu(x):
    c0 = float(np.sqrt(2.0 / np.pi))
    u = c0 * (x + 0.044715 * (x * x * x))
    return 0.5 * x * (1.0 + jnp.tanh(u))


def _dot(a, b):
    return jnp.dot(a, b, preferred_element_type=f32)


def _kernel(x_hbm, ckv_hbm, wq_hbm, wuk_hbm, wuv_hbm, wo_hbm, w1_hbm, w2_hbm, w3_hbm, w4_hbm, c_ref, wmod_hbm,
            out_hbm,
            x_s, ckv_s, hmod_s, wmod_s, mod_s, wo_s, w1_s, w2_s, w3_s, w4_s,
            wq_s, wuk_s, wuv_s, rq_s, ruk_s, ruv_s, w3t_s,
            q_s, kT_s, v_s, ctx_s, h_s, h1_s, acc_s, x2_s, out_s, y_s, ln1_s, sems, wsems, isems):
    u32 = jnp.uint32
    wq_pairs = wq_hbm.bitcast(u32)
    wuk_pairs = wuk_hbm.bitcast(u32)
    wuv_pairs = wuv_hbm.bitcast(u32)

    def pcopies(hh, sl):
        j = hh // 2
        return [pltpu.make_async_copy(wq_pairs.at[:, j, :], rq_s.at[sl], wsems.at[0, sl]),
                pltpu.make_async_copy(wuk_pairs.at[:, j, :], ruk_s.at[sl], wsems.at[1, sl]),
                pltpu.make_async_copy(wuv_pairs.at[:, j, :], ruv_s.at[sl], wsems.at[2, sl])]

    def unpack_weights(hh, sl):
        sh = jnp.asarray(16 * (1 - hh % 2)).astype(u32)
        for raw, dst in ((rq_s, wq_s.at[sl]), (ruk_s, wuk_s), (ruv_s, wuv_s)):
            bits = (raw[sl] << sh) & jnp.uint32(0xFFFF0000)
            dst[...] = pltpu.bitcast(bits, f32).astype(bf16)

    def wocopy(hh, sl):
        return pltpu.make_async_copy(wo_hbm.at[pl.ds(pl.multiple_of(hh * D, D), D), :], wo_s.at[sl], wsems.at[3, sl])

    def in_copies(i):
        r = pl.ds(pl.multiple_of(i * PB, PB), PB)
        return [pltpu.make_async_copy(x_hbm.at[r, :], x_s.at[r, :], isems.at[0, i]),
                pltpu.make_async_copy(ckv_hbm.at[r, :], ckv_s.at[r, :], isems.at[1, i])]

    cp_wmod0 = pltpu.make_async_copy(wmod_hbm.at[:, 0:2 * M], wmod_s.at[:, 0:2 * M], sems.at[2])
    cp_wmod1 = pltpu.make_async_copy(wmod_hbm.at[:, 2 * M:6 * M], wmod_s.at[:, 2 * M:6 * M], sems.at[3])
    cp_w1 = pltpu.make_async_copy(w1_hbm, w1_s, sems.at[4])
    cp_w2 = pltpu.make_async_copy(w2_hbm, w2_s, sems.at[5])
    cp_w3 = pltpu.make_async_copy(w3_hbm, w3t_s.at[0:F, :], sems.at[6])
    cp_w4 = pltpu.make_async_copy(w4_hbm, w4_s.at[0:F, :], sems.at[7])
    cp_out = pltpu.make_async_copy(out_s, out_hbm, sems.at[8])

    def kpiece(sl, rs):
        acc = None
        for t in range(NC):
            o = _dot(ckv_s[rs, t * 128:(t + 1) * 128], wuk_s[t * 128:(t + 1) * 128, :])
            acc = o if acc is None else acc + o
        if KNT:
            kT_s[rs, :] = acc.astype(bf16)
        else:
            kT_s[:, rs] = acc.astype(bf16).T

    def vpiece(sl, rs):
        acc = None
        for t in range(NC):
            o = _dot(ckv_s[rs, t * 128:(t + 1) * 128], wuv_s[t * 128:(t + 1) * 128, :])
            acc = o if acc is None else acc + o
        v_s[rs, :] = acc.astype(bf16)

    def qpiece(sl, rs):
        acc = None
        for t in range(NP):
            o = _dot(hmod_s[rs, t * 128:(t + 1) * 128], wq_s[sl, t * 128:(t + 1) * 128, :])
            acc = o if acc is None else acc + o
        q_s[rs, :] = (acc * QSCALE).astype(bf16)

    def prologue():
        cp_wmod0.start()
        for cp in pcopies(0, 0):
            cp.start()
        for i in range(LOOK):
            for cp in in_copies(i):
                cp.start()
        acc_s[...] = jnp.zeros((S, M), f32)
        h1_s[0:8, :] = jnp.zeros((8, M), f32)
        h1_s[S + 8:S + 16, :] = jnp.zeros((8, M), f32)
        if W3NT:
            w3t_s[F:FP, :] = jnp.zeros((FP - F, M), bf16)
        else:
            w3_s[:, F:FP] = jnp.zeros((M, FP - F), bf16)
        w4_s[F:FP, :] = jnp.zeros((FP - F, M), bf16)

        c = c_ref[...].astype(f32)
        sc = c * (1.0 / (1.0 + jnp.exp(-c)))
        sc8 = jnp.broadcast_to(sc, (16, M)).astype(bf16)
        cp_wmod0.wait()
        mod_s[:, 0:2 * M] = _dot(sc8, wmod_s[:, 0:2 * M])[0:8, :]
        sa = mod_s[0:1, 0:M]
        ca = mod_s[0:1, M:2 * M]
        for cp in pcopies(0, 0):
            cp.wait()
        unpack_weights(0, 0)

        def first_body(i, carry):
            r = pl.ds(pl.multiple_of(i * PB, PB), PB)
            for cp in in_copies(i):
                cp.wait()

            @pl.when(i + LOOK < S // PB)
            def _():
                for cp in in_copies(i + LOOK):
                    cp.start()

            @pl.when(i + LOOK == S // PB)
            def _():
                for cp in pcopies(1, 1):
                    cp.start()
                wocopy(0, 0).start()
            if PORD == 1:
                kpiece(0, r); vpiece(0, r)
            xb = x_s[r, :].astype(f32)
            hmod_s[r, :] = (_ln(xb) * (1.0 + ca) + sa).astype(bf16)
            if PORD == 0:
                kpiece(0, r); vpiece(0, r)
            qpiece(0, r)
            return carry
        lax.fori_loop(0, S // PB, first_body, 0)
        cp_wmod1.start()
        cp_w1.start(); cp_w2.start(); cp_w3.start(); cp_w4.start()
        return sc8

    sc8 = prologue()

    def head_body(h, carry):
        slot = h % 2
        nslot = 1 - slot
        def dma_turn():
            for cp in pcopies(jnp.minimum(h + 1, H - 1), nslot):
                cp.wait()
            wocopy(jnp.maximum(h - OPD, 0), slot).wait()
            for cp in pcopies(jnp.minimum(h + 2, H - 1), slot):
                cp.start()
            wocopy(jnp.minimum(h + 1 - OPD, H - 1), nslot).start()


        if DPOS == 0:
            dma_turn()
        row = lax.broadcasted_iota(jnp.int32, (128, 128), 0)
        col = lax.broadcasted_iota(jnp.int32, (128, 128), 1)
        causal = col <= row
        nq = S // BQ

        def qk_tiles(i, c0, cw):
            r0 = i * BQ
            q_i = q_s[r0:r0 + BQ, :]
            if KNT:
                s = lax.dot_general(q_i, kT_s[c0:c0 + cw, :], (((1,), (1,)), ((), ())), preferred_element_type=f32)
            else:
                s = _dot(q_i, kT_s[:, c0:c0 + cw])
            res = []
            for t in range(cw // 128):
                cc = c0 + t * 128
                st = s[:, t * 128:(t + 1) * 128]
                if cc + 128 > r0:
                    parts = []
                    for rr in range(BQ // 128):
                        rbase = r0 + rr * 128
                        if cc == rbase:
                            parts.append(jnp.where(causal, st[rr * 128:(rr + 1) * 128], NEG))
                        elif cc < rbase:
                            parts.append(st[rr * 128:(rr + 1) * 128])
                        else:
                            parts.append(jnp.full((128, 128), NEG, f32))
                    st = parts[0] if len(parts) == 1 else jnp.concatenate(parts, axis=0)
                res.append(st)
            return res

        def chunks(i, cwmax):
            L = (i + 1) * BQ
            return [(c0, min(cwmax, L - c0)) for c0 in range(0, L, cwmax)]

        def rowmax(tiles):
            m = tiles[0]
            for st in tiles[1:]:
                m = jnp.maximum(m, st)
            m = jnp.max(m, axis=-1, keepdims=True)
            return jnp.broadcast_to(m, (BQ, 128))

        order = list(range(nq - 1, -1, -1))
        pending = []

        def add_kq(i):
            if (i * BQ) % PR == 0:
                prs = slice(i * BQ, i * BQ + PR)
                pending.append(lambda: kpiece(nslot, prs))
                if i >= QDELAY:
                    pending.append(lambda: qpiece(nslot, prs))

        def add_v(i):
            if (i * BQ) % PR == 0:
                prs = slice(i * BQ, i * BQ + PR)
                pending.append(lambda: vpiece(nslot, prs))

        olds = []
        if QPOS == 0:
            for i_ in range(QDELAY - 1, -1, -1):
                qpiece(slot, slice(i_ * BQ, i_ * BQ + BQ))
            unpack_weights(jnp.minimum(h + 1, H - 1), nslot)
        cur = []
        for (c0, cw) in chunks(order[0], KC):
            cur += qk_tiles(order[0], c0, cw)
        if QPOS == 1:
            if DPOS == 1:
                dma_turn()
            for i_ in range(QDELAY - 1, -1, -1):
                qpiece(slot, slice(i_ * BQ, i_ * BQ + BQ))
            if DPOS == 2:
                dma_turn()
            unpack_weights(jnp.minimum(h + 1, H - 1), nslot)
        if QPOS == 2:
            for i_ in range(QDELAY - 1, -1, -1):
                pending.append(lambda i_=i_: qpiece(slot, slice(i_ * BQ, i_ * BQ + BQ)))
            pending.append(lambda: unpack_weights(jnp.minimum(h + 1, H - 1), nslot))
        mb = rowmax(cur)
        if EARLY:
            add_kq(order[0])
        if OPD:
            def opiece(rs):
                acc_s[rs, :] = acc_s[rs, :] + _dot(ctx_s[rs, :], wo_s[slot])
            for i_ in order:
                pending.append(lambda rs=slice(i_ * BQ, i_ * BQ + BQ): opiece(rs))
        for oi, i in enumerate(order):
            inext = order[oi + 1] if oi + 1 < nq else None
            nxt_chunks = chunks(inext, KC) if inext is not None else []
            nxt = []
            l = None
            acc = None
            ci = 0
            pv_chunks = chunks(i, PVC)
            npv = len(pv_chunks)
            if not THRX:
                olds = []
            for pi, (c0, cw) in enumerate(pv_chunks):
                def emit_qk():
                    nonlocal ci, nxt
                    while ci < len(nxt_chunks) and ci * npv < (pi + 1) * len(nxt_chunks):
                        nxt += qk_tiles(inext, *nxt_chunks[ci])
                        ci += 1
                if ORD == 0:
                    emit_qk()
                mbc = mb
                if THR and len(olds) >= THR:
                    mbc = mb + olds[-THR] * 0.0
                ps = [jnp.exp2(cur[t] - mbc) for t in range(c0 // 128, (c0 + cw) // 128)]
                pj = ps[0] if len(ps) == 1 else jnp.concatenate(ps, axis=1)
                pj = pj.astype(bf16)
                if LSUM == 1:
                    pf = pj.astype(f32)
                    ps = [pf[:, t * 128:(t + 1) * 128] for t in range(cw // 128)]
                if LSUM == 2:
                    for p in ps:
                        l = p if l is None else l + p
                else:
                    psum = ps[0]
                    for p in ps[1:]:
                        psum = psum + p
                    l = psum if l is None else l + psum
                o = _dot(pj, v_s[c0:c0 + cw, :])
                olds.append(o)
                acc = o if acc is None else acc + o
                if ORD == 1:
                    emit_qk()
                nemit = -(-len(pending) // (npv - pi))
                if OPD and oi < OPD_SPREAD:
                    nemit = min(nemit, -(-OPD_N // npv))
                for _ in range(nemit):
                    pending.pop(0)()
                if ORD == 2:
                    emit_qk()
            if EARLY and inext is not None:
                add_kq(inext)
            l = jnp.sum(l, axis=-1, keepdims=True)
            r = pl.reciprocal(l, approx=True)
            r = r * (2.0 - l * r)
            ctx = (acc * r).astype(bf16)
            rs = slice(i * BQ, i * BQ + BQ)
            if OPD:
                ctx_s[rs, :] = ctx
            else:
                acc_s[rs, :] = acc_s[rs, :] + _dot(ctx, wo_s[slot])
            if not EARLY:
                add_kq(i)
            add_v(i)
            if not PDELAY:
                while pending:
                    pending.pop(0)()
            if nxt:
                cur = nxt
                mb = rowmax(cur)
        while pending:
            pending.pop(0)()

        return carry

    lax.fori_loop(0, H, head_body, 0)
    for cp in pcopies(H - 1, (H - 1) % 2):
        cp.wait()
    wocopy(H - 1, H % 2).wait()

    def epilogue():
        cp_wmod1.wait()
        mod_s[:, 2 * M:6 * M] = _dot(sc8, wmod_s[:, 2 * M:6 * M])[0:8, :]
        cp_w1.wait(); cp_w2.wait(); cp_w3.wait(); cp_w4.wait()
        ga = mod_s[0:1, 2 * M:3 * M]
        sb = mod_s[0:1, 3 * M:4 * M]
        cb = mod_s[0:1, 4 * M:5 * M]
        gb = mod_s[0:1, 5 * M:6 * M]
        for t in range(0 if W3NT else FP // 128):
            n = min(128, F - t * 128)
            w3_s[:, t * 128:t * 128 + n] = w3t_s[t * 128:t * 128 + n, :].T

        lane = lax.broadcasted_iota(jnp.int32, (RB, 128), 1)

        def pass1(i):
            r0 = pl.multiple_of(i * RB, RB)
            r = pl.ds(r0, RB)
            att = acc_s[r, :]
            if OPD:
                att = att + _dot(ctx_s[r, :], wo_s[H % 2])
            x2 = x_s[r, :].astype(f32) + ga * att
            x2_s[r, :] = x2
            hb = _ln(x2) * (1.0 + cb) + sb
            h_s[r, :] = hb
            g = _gelu(_dot(_ln(hb).astype(bf16), w1_s[...]))
            h1_s[pl.ds(r0 + 8, RB), :] = g

        def stageB(i):
            r0 = pl.multiple_of(i * RB, RB)
            r = pl.ds(r0, RB)
            win = h1_s[pl.ds(r0, RB + 16), :]

            def sh(off, t):
                return win[8 + off:8 + off + RB, t * 128:(t + 1) * 128]
            t0 = sh(-1, 0)
            t1 = jnp.where(lane < 32, sh(-1, 1), sh(1, 1))
            t2 = jnp.where(lane < 64, sh(1, 2), sh(-2, 2))
            t3 = jnp.where(lane < 96, sh(-2, 3), sh(2, 3))
            t4 = sh(2, 4)
            g = jnp.concatenate([t0, t1, t2, t3, t4], axis=1).astype(bf16)
            x1 = h_s[r, :] + _dot(g, w2_s[...])
            y = x2_s[r, :] + gb * x1
            return y, _ln(x1).astype(bf16)

        def stageC(i, y, ln1):
            r0 = pl.multiple_of(i * RB, RB)
            r = pl.ds(r0, RB)
            pre = lax.dot_general(ln1, w3t_s[...], (((1,), (1,)), ((), ())), preferred_element_type=f32)
            u = _gelu(pre).astype(bf16)
            h2 = _dot(u, w4_s[...])
            if y is None:
                y = y_s[r, :]
            out_s[r, :] = (y + gb * h2).astype(bf16)
            pltpu.make_async_copy(out_s.at[r, :], out_hbm.at[r, :], sems.at[8]).start()

        def pass2(i, mid=None):
            y, ln1 = stageB(i)
            if mid is not None:
                mid()
            stageC(i, y, ln1)

        def stageB_store(i):
            r = pl.ds(pl.multiple_of(i * RB, RB), RB)
            y, ln1 = stageB(i)
            y_s[r, :] = y
            ln1_s[r, :] = ln1

        NB = S // RB
        if EPI == 0:
            def b1(i, carry):
                pass1(i)
                return carry
            lax.fori_loop(0, NB, b1, 0)

            def b2(i, carry):
                pass2(i)
                return carry
            lax.fori_loop(0, NB, b2, 0)
        elif EPI == 2:
            def b1(i, carry):
                pass1(i)
                return carry
            lax.fori_loop(0, 3, b1, 0)
            stageB_store(0)

            def b2(i, carry):
                r = pl.ds(pl.multiple_of(i * RB, RB), RB)
                if EORD == 0:
                    stageC(i, None, ln1_s[r, :])
                    stageB_store(jnp.minimum(i + 1, NB - 1))
                    pass1(jnp.minimum(i + 3, NB - 1))
                else:
                    ln1 = ln1_s[r, :]
                    stageB_store(jnp.minimum(i + 1, NB - 1))
                    pass1(jnp.minimum(i + 3, NB - 1))
                    stageC(i, None, ln1)
                return carry
            lax.fori_loop(0, NB, b2, 0)
        else:
            def b1(i, carry):
                pass1(i)
                return carry
            lax.fori_loop(0, 2, b1, 0)

            def b2(i, carry):
                pass2(i, lambda: pass1(jnp.minimum(i + 2, NB - 1)))
                return carry
            lax.fori_loop(0, NB, b2, 0)
        cp_out.wait()

    epilogue()


@jax.jit
def pallas_adaLN_cond__compressed_kv_cla__mixer_s_mlp__prompt_kernel(
        A_x, A_c_kv, A_w_q, A_w_uk, A_w_uv, A_w_o, B_x, B_w1, B_w2, B_w3, B_w4, c, w_mod):
    x = A_x.reshape(S, M)
    ckv = A_c_kv.reshape(S, DC)
    wq, wuk, wuv = A_w_q, A_w_uk, A_w_uv
    wo = A_w_o.reshape(H * D, M)
    hbm = pl.BlockSpec(memory_space=pltpu.HBM)
    out = pl.pallas_call(
        _kernel,
        grid=(1,),
        in_specs=[hbm, hbm, hbm, hbm, hbm, hbm, hbm, hbm, hbm, hbm,
                  pl.BlockSpec((1, M), lambda h: (0, 0)),
                  hbm],
        out_specs=hbm,
        out_shape=jax.ShapeDtypeStruct((S, M), bf16),
        scratch_shapes=[
            pltpu.VMEM((S, M), bf16),
            pltpu.VMEM((S, DC), bf16),
            pltpu.VMEM((S, M), bf16),
            pltpu.VMEM((M, 6 * M), bf16),
            pltpu.VMEM((8, 6 * M), f32),
            pltpu.VMEM((2, D, M), bf16),
            pltpu.VMEM((M, M), bf16),
            pltpu.VMEM((M, M), bf16),
            pltpu.VMEM((M, FP), bf16),
            pltpu.VMEM((FP, M), bf16),
            pltpu.VMEM((2, M, D), bf16),
            pltpu.VMEM((DC, D), bf16),
            pltpu.VMEM((DC, D), bf16),
            pltpu.VMEM((2, M, D), jnp.uint32),
            pltpu.VMEM((2, DC, D), jnp.uint32),
            pltpu.VMEM((2, DC, D), jnp.uint32),
            pltpu.VMEM((FP, M), bf16),
            pltpu.VMEM((S, D), bf16), pltpu.VMEM((S, D) if KNT else (D, S), bf16), pltpu.VMEM((S, D), bf16),
            pltpu.VMEM((S, D), bf16),
            pltpu.VMEM((S, M), f32),
            pltpu.VMEM((S + 16, M), f32),
            pltpu.VMEM((S, M), f32),
            pltpu.VMEM((S, M), f32),
            pltpu.VMEM((S, M), bf16),
            pltpu.VMEM((S, M), f32),
            pltpu.VMEM((S, M), bf16),
            pltpu.SemaphoreType.DMA((16,)),
            pltpu.SemaphoreType.DMA((4, 2)),
            pltpu.SemaphoreType.DMA((2, S // PB)),
        ],
        compiler_params=pltpu.CompilerParams(
            dimension_semantics=("arbitrary",),
            vmem_limit_bytes=110 * 1024 * 1024,
            flags=FLAGS,
        ),
    )(x, ckv, wq, wuk, wuv, wo, B_w1, B_w2, B_w3.T, B_w4, c, w_mod)
    return out.reshape(1, S, M)
```

```python
import numpy as np
import jax
import jax.numpy as jnp
from jax import lax
import jax.experimental.pallas as pl
import jax.experimental.pallas.tpu as pltpu

S = 2048
M = 640
H = 32
D = 128
DC = 512
F = 1728
FP = 1792

BQ = 128
KC = 1024
PVC = 1024
QDELAY = 8
PB = 256
SB = 128
RB = 512

LOG2E = 1.4426950408889634
QSCALE = float(D ** -0.5) * LOG2E
GELU_C = float(np.sqrt(2.0 / np.pi))
NEG = -1e30
NP = M // 128
NC = DC // 128
f32 = jnp.float32
bf16 = jnp.bfloat16
u32 = jnp.uint32


def _ln(x):
    m = jnp.mean(x, axis=-1, keepdims=True)
    xc = x - m
    v = jnp.mean(xc * xc, axis=-1, keepdims=True)
    return xc * lax.rsqrt(v + 1e-5)


def _gelu(x):
    u = GELU_C * (x + 0.044715 * (x * x * x))
    return 0.5 * x * (1.0 + jnp.tanh(u))


def _dot(a, b):
    return jnp.dot(a, b, preferred_element_type=f32)


def _dot_nt(a, b):
    return lax.dot_general(a, b, (((1,), (1,)), ((), ())), preferred_element_type=f32)


def _kernel(x_hbm, ckv_hbm, wq_hbm, wuk_hbm, wuv_hbm, wo_hbm, w1_hbm, w2_hbm, w3t_hbm, w4_hbm, c_ref, wmod_hbm,
            out_hbm,
            x_s, ckv_s, hmod_s, wmod_s, mod_s, wo_s, w1_s, w2_s, w3t_s, w4_s,
            wq_s, wuk_s, wuv_s, rq_s, ruk_s, ruv_s,
            q_s, k_s, v_s, acc_s, x2_s, h_s, h1_s, out_s,
            sems, wsems, isems):
    wq_pairs = wq_hbm.bitcast(u32)
    wuk_pairs = wuk_hbm.bitcast(u32)
    wuv_pairs = wuv_hbm.bitcast(u32)

    def pcopies(hh, sl):
        j = hh // 2
        return [pltpu.make_async_copy(wq_pairs.at[:, j, :], rq_s.at[sl], wsems.at[0, sl]),
                pltpu.make_async_copy(wuk_pairs.at[:, j, :], ruk_s.at[sl], wsems.at[1, sl]),
                pltpu.make_async_copy(wuv_pairs.at[:, j, :], ruv_s.at[sl], wsems.at[2, sl])]

    def unpack_weights(hh, sl):
        sh = jnp.asarray(16 * (1 - hh % 2)).astype(u32)
        for raw, dst in ((rq_s, wq_s.at[sl]), (ruk_s, wuk_s), (ruv_s, wuv_s)):
            bits = (raw[sl] << sh) & u32(0xFFFF0000)
            dst[...] = pltpu.bitcast(bits, f32).astype(bf16)

    def wocopy(hh, sl):
        return pltpu.make_async_copy(wo_hbm.at[pl.ds(pl.multiple_of(hh * D, D), D), :], wo_s.at[sl], wsems.at[3, sl])

    def in_copies(i):
        r = pl.ds(pl.multiple_of(i * PB, PB), PB)
        return [pltpu.make_async_copy(x_hbm.at[r, :], x_s.at[r, :], isems.at[0, i]),
                pltpu.make_async_copy(ckv_hbm.at[r, :], ckv_s.at[r, :], isems.at[1, i])]

    cp_wmod0 = pltpu.make_async_copy(wmod_hbm.at[:, 0:2 * M], wmod_s.at[:, 0:2 * M], sems.at[0])
    cp_wmod1 = pltpu.make_async_copy(wmod_hbm.at[:, 2 * M:6 * M], wmod_s.at[:, 2 * M:6 * M], sems.at[1])
    cp_w1 = pltpu.make_async_copy(w1_hbm, w1_s, sems.at[2])
    cp_w2 = pltpu.make_async_copy(w2_hbm, w2_s, sems.at[3])
    cp_w3 = pltpu.make_async_copy(w3t_hbm, w3t_s.at[0:F, :], sems.at[4])
    cp_w4 = pltpu.make_async_copy(w4_hbm, w4_s.at[0:F, :], sems.at[5])
    cp_out = pltpu.make_async_copy(out_s, out_hbm, sems.at[6])

    def proj(src_s, w_ref, nt, rs):
        acc = None
        for t in range(nt):
            o = _dot(src_s[rs, t * 128:(t + 1) * 128], w_ref[t * 128:(t + 1) * 128, :])
            acc = o if acc is None else acc + o
        return acc

    def kpiece(rs):
        k_s[rs, :] = proj(ckv_s, wuk_s, NC, rs).astype(bf16)

    def vpiece(rs):
        v_s[rs, :] = proj(ckv_s, wuv_s, NC, rs).astype(bf16)

    def qpiece(sl, rs):
        q_s[rs, :] = (proj(hmod_s, wq_s.at[sl], NP, rs) * QSCALE).astype(bf16)

    nb = S // PB
    LOOK = 2
    cp_wmod0.start()
    for cp in pcopies(0, 0):
        cp.start()
    for i in range(LOOK):
        for cp in in_copies(i):
            cp.start()
    acc_s[...] = jnp.zeros((S, M), f32)
    h1_s[0:8, :] = jnp.zeros((8, M), f32)
    h1_s[S + 8:S + 16, :] = jnp.zeros((8, M), f32)
    w3t_s[F:FP, :] = jnp.zeros((FP - F, M), bf16)
    w4_s[F:FP, :] = jnp.zeros((FP - F, M), bf16)

    c = c_ref[...].astype(f32)
    sc = c * (1.0 / (1.0 + jnp.exp(-c)))
    sc16 = jnp.broadcast_to(sc, (16, M)).astype(bf16)
    cp_wmod0.wait()
    mod_s[:, 0:2 * M] = _dot(sc16, wmod_s[:, 0:2 * M])[0:8, :]
    sa = mod_s[0:1, 0:M]
    ca = mod_s[0:1, M:2 * M]
    for cp in pcopies(0, 0):
        cp.wait()
    unpack_weights(0, 0)

    def first_body(i, carry):
        r = pl.ds(pl.multiple_of(i * PB, PB), PB)
        for cp in in_copies(i):
            cp.wait()

        @pl.when(i + LOOK < nb)
        def _():
            for cp in in_copies(i + LOOK):
                cp.start()

        @pl.when(i + LOOK == nb)
        def _():
            for cp in pcopies(1, 1):
                cp.start()
            wocopy(0, 0).start()

        kpiece(r)
        vpiece(r)
        hmod_s[r, :] = (_ln(x_s[r, :].astype(f32)) * (1.0 + ca) + sa).astype(bf16)
        qpiece(0, r)
        return carry

    lax.fori_loop(0, nb, first_body, 0)
    cp_wmod1.start()
    cp_w1.start()
    cp_w2.start()
    cp_w3.start()
    cp_w4.start()

    nq = S // BQ

    def head_body(h, carry):
        slot = h % 2
        nslot = 1 - slot
        for cp in pcopies(jnp.minimum(h + 1, H - 1), nslot):
            cp.wait()
        wocopy(h, slot).wait()
        for cp in pcopies(jnp.minimum(h + 2, H - 1), slot):
            cp.start()
        wocopy(jnp.minimum(h + 1, H - 1), nslot).start()

        row = lax.broadcasted_iota(jnp.int32, (128, 128), 0)
        col = lax.broadcasted_iota(jnp.int32, (128, 128), 1)
        causal = col <= row

        def blk(i):
            return slice(i * BQ, i * BQ + BQ)

        def chunks(i, cwmax):
            n = (i + 1) * BQ
            return [(c0, min(cwmax, n - c0)) for c0 in range(0, n, cwmax)]

        def qk_tiles(i, c0, cw):
            s = _dot_nt(q_s[blk(i), :], k_s[c0:c0 + cw, :])
            tiles = []
            for t in range(cw // 128):
                st = s[:, t * 128:(t + 1) * 128]
                if c0 + t * 128 == i * BQ:
                    st = jnp.where(causal, st, NEG)
                tiles.append(st)
            return tiles

        def rowmax(tiles):
            m = tiles[0]
            for st in tiles[1:]:
                m = jnp.maximum(m, st)
            return jnp.broadcast_to(jnp.max(m, axis=-1, keepdims=True), (BQ, 128))

        pending = []
        cur = []
        for (c0, cw) in chunks(nq - 1, KC):
            cur += qk_tiles(nq - 1, c0, cw)
        for i in range(QDELAY - 1, -1, -1):
            qpiece(slot, blk(i))
        unpack_weights(jnp.minimum(h + 1, H - 1), nslot)
        mb = rowmax(cur)

        for i in range(nq - 1, -1, -1):
            nxt_chunks = chunks(i - 1, KC) if i > 0 else []
            nxt = []
            l = None
            acc = None
            prev_o = None
            ci = 0
            pv_chunks = chunks(i, PVC)
            npv = len(pv_chunks)
            for pi, (c0, cw) in enumerate(pv_chunks):
                mbc = mb if prev_o is None else mb + prev_o * 0.0
                ps = [jnp.exp2(cur[t] - mbc) for t in range(c0 // 128, (c0 + cw) // 128)]
                pj = ps[0] if len(ps) == 1 else jnp.concatenate(ps, axis=1)
                psum = ps[0]
                for p in ps[1:]:
                    psum = psum + p
                l = psum if l is None else l + psum
                o = _dot(pj.astype(bf16), v_s[c0:c0 + cw, :])
                prev_o = o
                acc = o if acc is None else acc + o
                while ci < len(nxt_chunks) and ci * npv < (pi + 1) * len(nxt_chunks):
                    nxt += qk_tiles(i - 1, *nxt_chunks[ci])
                    ci += 1
                for _ in range(-(-len(pending) // (npv - pi))):
                    pending.pop(0)()
            l = jnp.sum(l, axis=-1, keepdims=True)
            r = pl.reciprocal(l, approx=True)
            r = r * (2.0 - l * r)
            ctx = (acc * r).astype(bf16)
            acc_s[blk(i), :] = acc_s[blk(i), :] + _dot(ctx, wo_s[slot])
            pending.append(lambda i=i: kpiece(blk(i)))
            if i >= QDELAY:
                pending.append(lambda i=i: qpiece(nslot, blk(i)))
            pending.append(lambda i=i: vpiece(blk(i)))
            if nxt:
                cur = nxt
                mb = rowmax(cur)
        while pending:
            pending.pop(0)()
        return carry

    lax.fori_loop(0, H, head_body, 0)
    for cp in pcopies(H - 1, (H - 1) % 2):
        cp.wait()
    wocopy(H - 1, H % 2).wait()

    cp_wmod1.wait()
    mod_s[:, 2 * M:6 * M] = _dot(sc16, wmod_s[:, 2 * M:6 * M])[0:8, :]
    cp_w1.wait()
    cp_w2.wait()
    cp_w3.wait()
    cp_w4.wait()
    ga = mod_s[0:1, 2 * M:3 * M]
    sb = mod_s[0:1, 3 * M:4 * M]
    cb = mod_s[0:1, 4 * M:5 * M]
    gb = mod_s[0:1, 5 * M:6 * M]

    for k in range(S // SB):
        r = slice(k * SB, (k + 1) * SB)
        x2 = x_s[r, :].astype(f32) + ga * acc_s[r, :]
        x2_s[r, :] = x2
        hb = _ln(x2) * (1.0 + cb) + sb
        h_s[r, :] = hb
        h1_s[k * SB + 8:(k + 1) * SB + 8, :] = _gelu(_dot(_ln(hb).astype(bf16), w1_s[...]))

    lane = lax.broadcasted_iota(jnp.int32, (SB, 128), 1)

    def mix(r0):
        r = pl.ds(r0, SB)
        win = h1_s[pl.ds(r0, SB + 16), :]

        def sh(off, t):
            return win[8 + off:8 + off + SB, t * 128:(t + 1) * 128]

        t0 = sh(-1, 0)
        t1 = jnp.where(lane < 32, sh(-1, 1), sh(1, 1))
        t2 = jnp.where(lane < 64, sh(1, 2), sh(-2, 2))
        t3 = jnp.where(lane < 96, sh(-2, 3), sh(2, 3))
        t4 = sh(2, 4)
        g = jnp.concatenate([t0, t1, t2, t3, t4], axis=1).astype(bf16)
        x1 = h_s[r, :] + _dot(g, w2_s[...])
        y = x2_s[r, :] + gb * x1
        return y, _ln(x1).astype(bf16)

    def mlp(r0, y, ln1):
        r = pl.ds(r0, SB)
        u = _gelu(_dot_nt(ln1, w3t_s[...])).astype(bf16)
        out_s[r, :] = (y + gb * _dot(u, w4_s[...])).astype(bf16)
        pltpu.make_async_copy(out_s.at[r, :], out_hbm.at[r, :], sems.at[6]).start()

    def pass2(i, carry):
        base = pl.multiple_of(i * RB, RB)
        starts = [pl.multiple_of(base + k * SB, SB) for k in range(RB // SB)]
        staged = [mix(r0) for r0 in starts]
        for r0, (y, ln1) in zip(starts, staged):
            mlp(r0, y, ln1)
        return carry

    lax.fori_loop(0, S // RB, pass2, 0)
    cp_out.wait()


@jax.jit
def pallas_adaLN_cond__compressed_kv_cla__mixer_s_mlp__prompt_kernel(
        A_x, A_c_kv, A_w_q, A_w_uk, A_w_uv, A_w_o, B_x, B_w1, B_w2, B_w3, B_w4, c, w_mod):
    del B_x
    hbm = pl.BlockSpec(memory_space=pltpu.HBM)
    out = pl.pallas_call(
        _kernel,
        grid=(1,),
        in_specs=[hbm, hbm, hbm, hbm, hbm, hbm, hbm, hbm, hbm, hbm,
                  pl.BlockSpec((1, M), lambda i: (0, 0)),
                  hbm],
        out_specs=hbm,
        out_shape=jax.ShapeDtypeStruct((S, M), bf16),
        scratch_shapes=[
            pltpu.VMEM((S, M), bf16),
            pltpu.VMEM((S, DC), bf16),
            pltpu.VMEM((S, M), bf16),
            pltpu.VMEM((M, 6 * M), bf16),
            pltpu.VMEM((8, 6 * M), f32),
            pltpu.VMEM((2, D, M), bf16),
            pltpu.VMEM((M, M), bf16),
            pltpu.VMEM((M, M), bf16),
            pltpu.VMEM((FP, M), bf16),
            pltpu.VMEM((FP, M), bf16),
            pltpu.VMEM((2, M, D), bf16),
            pltpu.VMEM((DC, D), bf16),
            pltpu.VMEM((DC, D), bf16),
            pltpu.VMEM((2, M, D), u32),
            pltpu.VMEM((2, DC, D), u32),
            pltpu.VMEM((2, DC, D), u32),
            pltpu.VMEM((S, D), bf16),
            pltpu.VMEM((S, D), bf16),
            pltpu.VMEM((S, D), bf16),
            pltpu.VMEM((S, M), f32),
            pltpu.VMEM((S, M), f32),
            pltpu.VMEM((S, M), f32),
            pltpu.VMEM((S + 16, M), f32),
            pltpu.VMEM((S, M), bf16),
            pltpu.SemaphoreType.DMA((7,)),
            pltpu.SemaphoreType.DMA((4, 2)),
            pltpu.SemaphoreType.DMA((2, S // PB)),
        ],
        compiler_params=pltpu.CompilerParams(
            dimension_semantics=("arbitrary",),
            vmem_limit_bytes=100 * 1024 * 1024,
        ),
    )(A_x.reshape(S, M), A_c_kv.reshape(S, DC), A_w_q, A_w_uk, A_w_uv, A_w_o.reshape(H * D, M),
      B_w1, B_w2, B_w3.T, B_w4, c, w_mod)
    return out.reshape(1, S, M)
```

```python
import functools

import numpy as np
import jax
import jax.numpy as jnp
from jax import lax
import jax.experimental.pallas as pl
import jax.experimental.pallas.tpu as pltpu

S = 2048
M = 640
H = 32
D = 128
DC = 512
F = 1728
FP = 1792

BQ = 128
KC = 1024
PVC = 1024
QDELAY = 12
VDELAY = 8
PB = 256
SB = 128
RB = 512

LOG2E = 1.4426950408889634
QSCALE = float(D ** -0.5) * LOG2E
GELU_C = float(np.sqrt(2.0 / np.pi))
NEG = -1e30
NP = M // 128
NC = DC // 128
f32 = jnp.float32
bf16 = jnp.bfloat16
u32 = jnp.uint32


def _ln(x):
    m = jnp.mean(x, axis=-1, keepdims=True)
    xc = x - m
    v = jnp.mean(xc * xc, axis=-1, keepdims=True)
    return xc * lax.rsqrt(v + 1e-5)


def _gelu(x):
    u = x * (GELU_C + (GELU_C * 0.044715) * (x * x))
    hx = 0.5 * x
    return hx + hx * jnp.tanh(u)


def _dot(a, b):
    return jnp.dot(a, b, preferred_element_type=f32)


def _dot_nt(a, b):
    return lax.dot_general(a, b, (((1,), (1,)), ((), ())), preferred_element_type=f32)


def _kernel(x_hbm, ckv_hbm, wq_hbm, wuk_hbm, wuv_hbm, wo_hbm, w1_hbm, w2_hbm, w3t_hbm, w4_hbm, c_ref, wmod_hbm,
            out_hbm,
            x_s, ckv_s, hmod_s, wmod_s, mod_s, wo_s, w1_s, w2_s, w3t_s, w4_s,
            wq_s, wuk_s, wuv_s, rq_s, ruk_s, ruv_s,
            q_s, k_s, v_s, acc_s, x2_s, h_s, h1_s, out_s,
            sems, wsems, isems):
    wq_pairs = wq_hbm.bitcast(u32)
    wuk_pairs = wuk_hbm.bitcast(u32)
    wuv_pairs = wuv_hbm.bitcast(u32)

    def pcopies(hh, sl):
        j = hh // 2
        return [pltpu.make_async_copy(wq_pairs.at[:, j, :], rq_s.at[sl], wsems.at[0, sl]),
                pltpu.make_async_copy(wuk_pairs.at[:, j, :], ruk_s.at[sl], wsems.at[1, sl]),
                pltpu.make_async_copy(wuv_pairs.at[:, j, :], ruv_s.at[sl], wsems.at[2, sl])]

    def unpack_weights(hh, sl):
        sh = jnp.asarray(16 * (1 - hh % 2)).astype(u32)
        for raw, dst in ((rq_s, wq_s), (ruk_s, wuk_s), (ruv_s, wuv_s)):
            bits = (raw[sl] << sh) & u32(0xFFFF0000)
            dst[...] = pltpu.bitcast(bits, f32).astype(bf16)

    def wocopy(hh, sl):
        return pltpu.make_async_copy(wo_hbm.at[pl.ds(pl.multiple_of(hh * D, D), D), :], wo_s.at[sl], wsems.at[3, sl])

    def in_copies(i):
        r = pl.ds(pl.multiple_of(i * PB, PB), PB)
        return [pltpu.make_async_copy(x_hbm.at[r, :], x_s.at[r, :], isems.at[0, i]),
                pltpu.make_async_copy(ckv_hbm.at[r, :], ckv_s.at[r, :], isems.at[1, i])]

    cp_wmod0 = pltpu.make_async_copy(wmod_hbm.at[:, 0:2 * M], wmod_s.at[:, 0:2 * M], sems.at[0])
    cp_wmod1 = pltpu.make_async_copy(wmod_hbm.at[:, 2 * M:6 * M], wmod_s.at[:, 2 * M:6 * M], sems.at[1])
    cp_w1 = pltpu.make_async_copy(w1_hbm, w1_s, sems.at[2])
    cp_w2 = pltpu.make_async_copy(w2_hbm, w2_s, sems.at[3])
    cp_w3 = pltpu.make_async_copy(w3t_hbm, w3t_s.at[0:F, :], sems.at[4])
    cp_w4 = pltpu.make_async_copy(w4_hbm, w4_s.at[0:F, :], sems.at[5])
    cp_out = pltpu.make_async_copy(out_s, out_hbm, sems.at[6])

    def proj(src_s, w_ref, nt, rs):
        acc = None
        for t in range(nt):
            o = _dot(src_s[rs, t * 128:(t + 1) * 128], w_ref[t * 128:(t + 1) * 128, :])
            acc = o if acc is None else acc + o
        return acc

    def kpiece(rs):
        k_s[rs, :] = proj(ckv_s, wuk_s, NC, rs).astype(bf16)

    def vpiece(rs):
        v_s[rs, :] = proj(ckv_s, wuv_s, NC, rs).astype(bf16)

    def qpiece(rs):
        q_s[rs, :] = (proj(hmod_s, wq_s, NP, rs) * QSCALE).astype(bf16)

    nb = S // PB
    LOOK = 2
    cp_wmod0.start()
    for cp in pcopies(0, 0):
        cp.start()
    for i in range(LOOK):
        for cp in in_copies(i):
            cp.start()
    acc_s[...] = jnp.zeros((S, M), f32)
    h1_s[0:8, :] = jnp.zeros((8, M), f32)
    h1_s[S + 8:S + 16, :] = jnp.zeros((8, M), f32)
    w3t_s[F:FP, :] = jnp.zeros((FP - F, M), bf16)
    w4_s[F:FP, :] = jnp.zeros((FP - F, M), bf16)

    c = c_ref[...].astype(f32)
    sc = c * (1.0 / (1.0 + jnp.exp(-c)))
    sc16 = jnp.broadcast_to(sc, (16, M)).astype(bf16)
    cp_wmod0.wait()
    mod_s[:, 0:2 * M] = _dot(sc16, wmod_s[:, 0:2 * M])[0:8, :]
    sa = mod_s[0:1, 0:M]
    ca = mod_s[0:1, M:2 * M]
    for cp in pcopies(0, 0):
        cp.wait()
    unpack_weights(0, 0)

    def first_body(i, carry, do_v, do_q):
        r = pl.ds(pl.multiple_of(i * PB, PB), PB)
        for cp in in_copies(i):
            cp.wait()

        @pl.when(i + LOOK < nb)
        def _():
            for cp in in_copies(i + LOOK):
                cp.start()

        @pl.when(i + LOOK == nb)
        def _():
            for cp in pcopies(1, 1):
                cp.start()
            wocopy(0, 0).start()

        kpiece(r)
        if do_v:
            vpiece(r)
        hmod_s[r, :] = (_ln(x_s[r, :].astype(f32)) * (1.0 + ca) + sa).astype(bf16)
        if do_q:
            qpiece(r)
        return carry

    nv, nqd = VDELAY * BQ // PB, QDELAY * BQ // PB
    lax.fori_loop(0, nv, functools.partial(first_body, do_v=False, do_q=False), 0)
    lax.fori_loop(nv, nqd, functools.partial(first_body, do_v=True, do_q=False), 0)
    lax.fori_loop(nqd, nb, functools.partial(first_body, do_v=True, do_q=True), 0)
    cp_wmod1.start()
    cp_w1.start()
    cp_w2.start()
    cp_w3.start()
    cp_w4.start()

    nq = S // BQ

    def head_body(h, carry):
        slot = h % 2
        nslot = 1 - slot
        for cp in pcopies(jnp.minimum(h + 1, H - 1), nslot):
            cp.wait()
        wocopy(h, slot).wait()
        for cp in pcopies(jnp.minimum(h + 2, H - 1), slot):
            cp.start()
        wocopy(jnp.minimum(h + 1, H - 1), nslot).start()

        row = lax.broadcasted_iota(jnp.int32, (128, 128), 0)
        col = lax.broadcasted_iota(jnp.int32, (128, 128), 1)
        causal = col <= row

        def blk(i):
            return slice(i * BQ, i * BQ + BQ)

        def chunks(i, cwmax):
            n = (i + 1) * BQ
            return [(c0, min(cwmax, n - c0)) for c0 in range(0, n, cwmax)]

        def qk_tiles(i, c0, cw):
            s = _dot_nt(q_s[blk(i), :], k_s[c0:c0 + cw, :])
            tiles = []
            for t in range(cw // 128):
                st = s[:, t * 128:(t + 1) * 128]
                if c0 + t * 128 == i * BQ:
                    st = jnp.where(causal, st, NEG)
                tiles.append(st)
            return tiles

        def rowmax(tiles):
            m = tiles[0]
            for st in tiles[1:]:
                m = jnp.maximum(m, st)
            return jnp.broadcast_to(jnp.max(m, axis=-1, keepdims=True), (BQ, 128))

        pending = []
        for i in range(VDELAY - 1, -1, -1):
            vpiece(blk(i))
        cur = []
        for (c0, cw) in chunks(nq - 1, KC):
            cur += qk_tiles(nq - 1, c0, cw)
        for i in range(QDELAY - 1, -1, -1):
            qpiece(blk(i))
        unpack_weights(jnp.minimum(h + 1, H - 1), nslot)
        mb = rowmax(cur)

        for i in range(nq - 1, -1, -1):
            nxt_chunks = chunks(i - 1, KC) if i > 0 else []
            nxt = []
            l = None
            acc = None
            prev_o = None
            ci = 0
            pv_chunks = chunks(i, PVC)
            npv = len(pv_chunks)
            for pi, (c0, cw) in enumerate(pv_chunks):
                mbc = mb if prev_o is None else mb + prev_o * 0.0
                ps = [jnp.exp2(cur[t] - mbc) for t in range(c0 // 128, (c0 + cw) // 128)]
                pj = ps[0] if len(ps) == 1 else jnp.concatenate(ps, axis=1)
                psum = ps[0]
                for p in ps[1:]:
                    psum = psum + p
                l = psum if l is None else l + psum
                o = _dot(pj.astype(bf16), v_s[c0:c0 + cw, :])
                prev_o = o
                acc = o if acc is None else acc + o
                while ci < len(nxt_chunks) and ci * npv < (pi + 1) * len(nxt_chunks):
                    nxt += qk_tiles(i - 1, *nxt_chunks[ci])
                    ci += 1
                for _ in range(-(-len(pending) // (npv - pi))):
                    pending.pop(0)()
            l = jnp.sum(l, axis=-1, keepdims=True)
            r = pl.reciprocal(l, approx=True)
            r = r * (2.0 - l * r)
            ctx = (acc * r).astype(bf16)
            acc_s[blk(i), :] = acc_s[blk(i), :] + _dot(ctx, wo_s[slot])
            pending.append(lambda i=i: kpiece(blk(i)))
            if i >= QDELAY:
                pending.append(lambda i=i: qpiece(blk(i)))
            if i >= VDELAY:
                pending.append(lambda i=i: vpiece(blk(i)))
            if nxt:
                cur = nxt
                mb = rowmax(cur)
        while pending:
            pending.pop(0)()
        return carry

    lax.fori_loop(0, H, head_body, 0)
    for cp in pcopies(H - 1, (H - 1) % 2):
        cp.wait()
    wocopy(H - 1, H % 2).wait()

    cp_wmod1.wait()
    mod_s[:, 2 * M:6 * M] = _dot(sc16, wmod_s[:, 2 * M:6 * M])[0:8, :]
    cp_w1.wait()
    cp_w2.wait()
    cp_w3.wait()
    cp_w4.wait()
    ga = mod_s[0:1, 2 * M:3 * M]
    sb = mod_s[0:1, 3 * M:4 * M]
    cb = mod_s[0:1, 4 * M:5 * M]
    gb = mod_s[0:1, 5 * M:6 * M]

    for k in range(S // SB):
        r = slice(k * SB, (k + 1) * SB)
        x2 = x_s[r, :].astype(f32) + ga * acc_s[r, :]
        x2_s[r, :] = x2
        hb = _ln(x2) * (1.0 + cb) + sb
        h_s[r, :] = hb
        h1_s[k * SB + 8:(k + 1) * SB + 8, :] = _gelu(_dot(_ln(hb).astype(bf16), w1_s[...]))

    lane = lax.broadcasted_iota(jnp.int32, (SB, 128), 1)

    def mix(r0):
        r = pl.ds(r0, SB)
        win = h1_s[pl.ds(r0, SB + 16), :]

        def sh(off, t):
            return win[8 + off:8 + off + SB, t * 128:(t + 1) * 128]

        t0 = sh(-1, 0)
        t1 = jnp.where(lane < 32, sh(-1, 1), sh(1, 1))
        t2 = jnp.where(lane < 64, sh(1, 2), sh(-2, 2))
        t3 = jnp.where(lane < 96, sh(-2, 3), sh(2, 3))
        t4 = sh(2, 4)
        g = jnp.concatenate([t0, t1, t2, t3, t4], axis=1).astype(bf16)
        x1 = h_s[r, :] + _dot(g, w2_s[...])
        y = x2_s[r, :] + gb * x1
        return y, _ln(x1).astype(bf16)

    def mlp(r0, y, ln1):
        r = pl.ds(r0, SB)
        u = _gelu(_dot_nt(ln1, w3t_s[...])).astype(bf16)
        out_s[r, :] = (y + gb * _dot(u, w4_s[...])).astype(bf16)
        pltpu.make_async_copy(out_s.at[r, :], out_hbm.at[r, :], sems.at[6]).start()

    def pass2(i, carry):
        base = pl.multiple_of(i * RB, RB)
        starts = [pl.multiple_of(base + k * SB, SB) for k in range(RB // SB)]
        staged = [mix(r0) for r0 in starts]
        for r0, (y, ln1) in zip(starts, staged):
            mlp(r0, y, ln1)
        return carry

    lax.fori_loop(0, S // RB, pass2, 0)
    cp_out.wait()


@jax.jit
def pallas_adaLN_cond__compressed_kv_cla__mixer_s_mlp__prompt_kernel(
        A_x, A_c_kv, A_w_q, A_w_uk, A_w_uv, A_w_o, B_x, B_w1, B_w2, B_w3, B_w4, c, w_mod):
    del B_x
    hbm = pl.BlockSpec(memory_space=pltpu.HBM)
    out = pl.pallas_call(
        _kernel,
        grid=(1,),
        in_specs=[hbm, hbm, hbm, hbm, hbm, hbm, hbm, hbm, hbm, hbm,
                  pl.BlockSpec((1, M), lambda i: (0, 0)),
                  hbm],
        out_specs=hbm,
        out_shape=jax.ShapeDtypeStruct((S, M), bf16),
        scratch_shapes=[
            pltpu.VMEM((S, M), bf16),
            pltpu.VMEM((S, DC), bf16),
            pltpu.VMEM((S, M), bf16),
            pltpu.VMEM((M, 6 * M), bf16),
            pltpu.VMEM((8, 6 * M), f32),
            pltpu.VMEM((2, D, M), bf16),
            pltpu.VMEM((M, M), bf16),
            pltpu.VMEM((M, M), bf16),
            pltpu.VMEM((FP, M), bf16),
            pltpu.VMEM((FP, M), bf16),
            pltpu.VMEM((M, D), bf16),
            pltpu.VMEM((DC, D), bf16),
            pltpu.VMEM((DC, D), bf16),
            pltpu.VMEM((2, M, D), u32),
            pltpu.VMEM((2, DC, D), u32),
            pltpu.VMEM((2, DC, D), u32),
            pltpu.VMEM((S, D), bf16),
            pltpu.VMEM((S, D), bf16),
            pltpu.VMEM((S, D), bf16),
            pltpu.VMEM((S, M), f32),
            pltpu.VMEM((S, M), f32),
            pltpu.VMEM((S, M), f32),
            pltpu.VMEM((S + 16, M), f32),
            pltpu.VMEM((S, M), bf16),
            pltpu.SemaphoreType.DMA((7,)),
            pltpu.SemaphoreType.DMA((4, 2)),
            pltpu.SemaphoreType.DMA((2, S // PB)),
        ],
        compiler_params=pltpu.CompilerParams(
            dimension_semantics=("arbitrary",),
            vmem_limit_bytes=100 * 1024 * 1024,
            flags={"XLA_TPU_RESCHEDULE_DMA_DONES": True},
        ),
    )(A_x.reshape(S, M), A_c_kv.reshape(S, DC), A_w_q, A_w_uk, A_w_uv, A_w_o.reshape(H * D, M),
      B_w1, B_w2, B_w3.T, B_w4, c, w_mod)
    return out.reshape(1, S, M)
```

```python
import functools

import numpy as np
import jax
import jax.numpy as jnp
from jax import lax
import jax.experimental.pallas as pl
import jax.experimental.pallas.tpu as pltpu

S = 2048
M = 640
H = 32
D = 128
DC = 512
F = 1728
FP = 1792

BQ = 128
KC = 1024
PVC = 1024
QDELAY = 12
VDELAY = 8
PB = 256
SB = 128
RB = 512

LOG2E = 1.4426950408889634
QSCALE = float(D ** -0.5) * LOG2E
GELU_C = float(np.sqrt(2.0 / np.pi))
NEG = -1e30
NP = M // 128
NC = DC // 128
f32 = jnp.float32
bf16 = jnp.bfloat16
u32 = jnp.uint32


def _ln(x):
    m = jnp.mean(x, axis=-1, keepdims=True)
    xc = x - m
    v = jnp.mean(xc * xc, axis=-1, keepdims=True)
    return xc * lax.rsqrt(v + 1e-5)


def _gelu(x):
    u = x * (GELU_C + (GELU_C * 0.044715) * (x * x))
    hx = 0.5 * x
    return hx + hx * jnp.tanh(u)


def _dot(a, b):
    return jnp.dot(a, b, preferred_element_type=f32)


def _dot_nt(a, b):
    return lax.dot_general(a, b, (((1,), (1,)), ((), ())), preferred_element_type=f32)


def _kernel(x_hbm, ckv_hbm, wq_hbm, wuk_hbm, wuv_hbm, wo_hbm, w1_hbm, w2_hbm, w3t_hbm, w4_hbm, c_ref, wmod_hbm,
            out_hbm,
            x_s, ckv_s, hmod_s, wmod_s, mod_s, wo_s, w1_s, w2_s, w3t_s, w4_s,
            wq_s, wuk_s, wuv_s, rq_s, ruk_s, ruv_s,
            q_s, k_s, v_s, acc_s, x2_s, h_s, h1_s, out_s,
            sems, wsems, isems):
    wq_pairs = wq_hbm.bitcast(u32)
    wuk_pairs = wuk_hbm.bitcast(u32)
    wuv_pairs = wuv_hbm.bitcast(u32)

    def pcopies(hh, sl):
        j = hh // 2
        return [pltpu.make_async_copy(wq_pairs.at[:, j, :], rq_s.at[sl], wsems.at[0, sl]),
                pltpu.make_async_copy(wuk_pairs.at[:, j, :], ruk_s.at[sl], wsems.at[1, sl]),
                pltpu.make_async_copy(wuv_pairs.at[:, j, :], ruv_s.at[sl], wsems.at[2, sl])]

    def unpack_weights(hh, sl):
        sh = jnp.asarray(16 * (1 - hh % 2)).astype(u32)
        for raw, dst in ((rq_s, wq_s), (ruk_s, wuk_s), (ruv_s, wuv_s)):
            bits = (raw[sl] << sh) & u32(0xFFFF0000)
            dst[...] = pltpu.bitcast(bits, f32).astype(bf16)

    def wocopy(hh, sl):
        return pltpu.make_async_copy(wo_hbm.at[pl.ds(pl.multiple_of(hh * D, D), D), :], wo_s.at[sl], wsems.at[3, sl])

    def in_copies(i):
        r = pl.ds(pl.multiple_of(i * PB, PB), PB)
        return [pltpu.make_async_copy(x_hbm.at[r, :], x_s.at[r, :], isems.at[0, i]),
                pltpu.make_async_copy(ckv_hbm.at[r, :], ckv_s.at[r, :], isems.at[1, i])]

    cp_wmod0 = pltpu.make_async_copy(wmod_hbm.at[:, 0:2 * M], wmod_s.at[:, 0:2 * M], sems.at[0])
    cp_wmod1 = pltpu.make_async_copy(wmod_hbm.at[:, 2 * M:6 * M], wmod_s.at[:, 2 * M:6 * M], sems.at[1])
    cp_w1 = pltpu.make_async_copy(w1_hbm, w1_s, sems.at[2])
    cp_w2 = pltpu.make_async_copy(w2_hbm, w2_s, sems.at[3])
    cp_w3 = pltpu.make_async_copy(w3t_hbm, w3t_s.at[0:F, :], sems.at[4])
    cp_w4 = pltpu.make_async_copy(w4_hbm, w4_s.at[0:F, :], sems.at[5])
    cp_out = pltpu.make_async_copy(out_s, out_hbm, sems.at[6])

    def proj(src_s, w_ref, nt, rs):
        acc = None
        for t in range(nt):
            o = _dot(src_s[rs, t * 128:(t + 1) * 128], w_ref[t * 128:(t + 1) * 128, :])
            acc = o if acc is None else acc + o
        return acc

    def kpiece(rs):
        k_s[rs, :] = proj(ckv_s, wuk_s, NC, rs).astype(bf16)

    def vpiece(rs):
        v_s[rs, :] = proj(ckv_s, wuv_s, NC, rs).astype(bf16)

    def qpiece(rs):
        q_s[rs, :] = (proj(hmod_s, wq_s, NP, rs) * QSCALE).astype(bf16)

    nb = S // PB
    LOOK = 2
    cp_wmod0.start()
    for cp in pcopies(0, 0):
        cp.start()
    for i in range(LOOK):
        for cp in in_copies(i):
            cp.start()
    acc_s[...] = jnp.zeros((S, M), f32)
    h1_s[0:8, :] = jnp.zeros((8, M), f32)
    h1_s[S + 8:S + 16, :] = jnp.zeros((8, M), f32)
    w3t_s[F:FP, :] = jnp.zeros((FP - F, M), bf16)
    w4_s[F:FP, :] = jnp.zeros((FP - F, M), bf16)

    c = c_ref[...].astype(f32)
    sc = c * (1.0 / (1.0 + jnp.exp(-c)))
    sc16 = jnp.broadcast_to(sc, (16, M)).astype(bf16)
    cp_wmod0.wait()
    mod_s[:, 0:2 * M] = _dot(sc16, wmod_s[:, 0:2 * M])[0:8, :]
    sa = mod_s[0:1, 0:M]
    ca = mod_s[0:1, M:2 * M]
    for cp in pcopies(0, 0):
        cp.wait()
    unpack_weights(0, 0)

    def first_body(i, carry, do_v, do_q):
        r = pl.ds(pl.multiple_of(i * PB, PB), PB)
        for cp in in_copies(i):
            cp.wait()

        @pl.when(i + LOOK < nb)
        def _():
            for cp in in_copies(i + LOOK):
                cp.start()

        @pl.when(i + LOOK == nb)
        def _():
            for cp in pcopies(1, 1):
                cp.start()
            wocopy(0, 0).start()

        kpiece(r)
        if do_v:
            vpiece(r)
        hmod_s[r, :] = (_ln(x_s[r, :].astype(f32)) * (1.0 + ca) + sa).astype(bf16)
        if do_q:
            qpiece(r)
        return carry

    nv, nqd = VDELAY * BQ // PB, QDELAY * BQ // PB
    lax.fori_loop(0, nv, functools.partial(first_body, do_v=False, do_q=False), 0)
    lax.fori_loop(nv, nqd, functools.partial(first_body, do_v=True, do_q=False), 0)
    lax.fori_loop(nqd, nb, functools.partial(first_body, do_v=True, do_q=True), 0)
    cp_wmod1.start()
    cp_w1.start()
    cp_w2.start()
    cp_w3.start()
    cp_w4.start()

    nq = S // BQ

    def head_body(h):
        slot = h % 2
        nslot = 1 - slot
        for cp in pcopies(jnp.minimum(h + 1, H - 1), nslot):
            cp.wait()
        wocopy(h, slot).wait()
        for cp in pcopies(jnp.minimum(h + 2, H - 1), slot):
            cp.start()
        wocopy(jnp.minimum(h + 1, H - 1), nslot).start()

        row = lax.broadcasted_iota(jnp.int32, (128, 128), 0)
        col = lax.broadcasted_iota(jnp.int32, (128, 128), 1)
        causal = col <= row

        def blk(i):
            return slice(i * BQ, i * BQ + BQ)

        def chunks(i, cwmax):
            n = (i + 1) * BQ
            return [(c0, min(cwmax, n - c0)) for c0 in range(0, n, cwmax)]

        def qk_tiles(i, c0, cw):
            s = _dot_nt(q_s[blk(i), :], k_s[c0:c0 + cw, :])
            tiles = []
            for t in range(cw // 128):
                st = s[:, t * 128:(t + 1) * 128]
                if c0 + t * 128 == i * BQ:
                    st = jnp.where(causal, st, NEG)
                tiles.append(st)
            return tiles

        def rowmax(tiles):
            m = tiles[0]
            for st in tiles[1:]:
                m = jnp.maximum(m, st)
            return jnp.broadcast_to(jnp.max(m, axis=-1, keepdims=True), (BQ, 128))

        pending = []
        for i in range(VDELAY - 1, -1, -1):
            vpiece(blk(i))
        cur = []
        for (c0, cw) in chunks(nq - 1, KC):
            cur += qk_tiles(nq - 1, c0, cw)
        for i in range(QDELAY - 1, -1, -1):
            qpiece(blk(i))
        unpack_weights(jnp.minimum(h + 1, H - 1), nslot)
        mb = rowmax(cur)

        for i in range(nq - 1, -1, -1):
            nxt_chunks = chunks(i - 1, KC) if i > 0 else []
            nxt = []
            l = None
            acc = None
            prev_o = None
            ci = 0
            pv_chunks = chunks(i, PVC)
            npv = len(pv_chunks)
            for pi, (c0, cw) in enumerate(pv_chunks):
                mbc = mb if prev_o is None else mb + prev_o * 0.0
                ps = [jnp.exp2(cur[t] - mbc) for t in range(c0 // 128, (c0 + cw) // 128)]
                pj = ps[0] if len(ps) == 1 else jnp.concatenate(ps, axis=1)
                psum = ps[0]
                for p in ps[1:]:
                    psum = psum + p
                l = psum if l is None else l + psum
                o = _dot(pj.astype(bf16), v_s[c0:c0 + cw, :])
                prev_o = o
                acc = o if acc is None else acc + o
                while ci < len(nxt_chunks) and ci * npv < (pi + 1) * len(nxt_chunks):
                    nxt += qk_tiles(i - 1, *nxt_chunks[ci])
                    ci += 1
                for _ in range(-(-len(pending) // (npv - pi))):
                    pending.pop(0)()
            l = jnp.sum(l, axis=-1, keepdims=True)
            r = pl.reciprocal(l, approx=True)
            r = r * (2.0 - l * r)
            ctx = (acc * r).astype(bf16)
            acc_s[blk(i), :] = acc_s[blk(i), :] + _dot(ctx, wo_s[slot])
            pending.append(lambda i=i: kpiece(blk(i)))
            if i >= QDELAY:
                pending.append(lambda i=i: qpiece(blk(i)))
            if i >= VDELAY:
                pending.append(lambda i=i: vpiece(blk(i)))
            if nxt:
                cur = nxt
                mb = rowmax(cur)
        while pending:
            pending.pop(0)()

    def two_heads(g, carry):
        head_body(2 * g)
        head_body(2 * g + 1)
        return carry

    lax.fori_loop(0, H // 2, two_heads, 0)
    for cp in pcopies(H - 1, (H - 1) % 2):
        cp.wait()
    wocopy(H - 1, H % 2).wait()

    cp_wmod1.wait()
    mod_s[:, 2 * M:6 * M] = _dot(sc16, wmod_s[:, 2 * M:6 * M])[0:8, :]
    cp_w1.wait()
    cp_w2.wait()
    cp_w3.wait()
    cp_w4.wait()
    ga = mod_s[0:1, 2 * M:3 * M]
    sb = mod_s[0:1, 3 * M:4 * M]
    cb = mod_s[0:1, 4 * M:5 * M]
    gb = mod_s[0:1, 5 * M:6 * M]

    for k in range(S // SB):
        r = slice(k * SB, (k + 1) * SB)
        x2 = x_s[r, :].astype(f32) + ga * acc_s[r, :]
        x2_s[r, :] = x2
        hb = _ln(x2) * (1.0 + cb) + sb
        h_s[r, :] = hb
        h1_s[k * SB + 8:(k + 1) * SB + 8, :] = _gelu(_dot(_ln(hb).astype(bf16), w1_s[...]))

    lane = lax.broadcasted_iota(jnp.int32, (SB, 128), 1)

    def mix(r0):
        r = pl.ds(r0, SB)
        win = h1_s[pl.ds(r0, SB + 16), :]

        def sh(off, t):
            return win[8 + off:8 + off + SB, t * 128:(t + 1) * 128]

        t0 = sh(-1, 0)
        t1 = jnp.where(lane < 32, sh(-1, 1), sh(1, 1))
        t2 = jnp.where(lane < 64, sh(1, 2), sh(-2, 2))
        t3 = jnp.where(lane < 96, sh(-2, 3), sh(2, 3))
        t4 = sh(2, 4)
        g = jnp.concatenate([t0, t1, t2, t3, t4], axis=1).astype(bf16)
        x1 = h_s[r, :] + _dot(g, w2_s[...])
        y = x2_s[r, :] + gb * x1
        return y, _ln(x1).astype(bf16)

    def mlp(r0, y, ln1):
        r = pl.ds(r0, SB)
        u = _gelu(_dot_nt(ln1, w3t_s[...])).astype(bf16)
        out_s[r, :] = (y + gb * _dot(u, w4_s[...])).astype(bf16)
        pltpu.make_async_copy(out_s.at[r, :], out_hbm.at[r, :], sems.at[6]).start()

    def pass2(i, carry):
        base = pl.multiple_of(i * RB, RB)
        starts = [pl.multiple_of(base + k * SB, SB) for k in range(RB // SB)]
        staged = [mix(r0) for r0 in starts]
        for r0, (y, ln1) in zip(starts, staged):
            mlp(r0, y, ln1)
        return carry

    lax.fori_loop(0, S // RB, pass2, 0)
    cp_out.wait()


@jax.jit
def pallas_adaLN_cond__compressed_kv_cla__mixer_s_mlp__prompt_kernel(
        A_x, A_c_kv, A_w_q, A_w_uk, A_w_uv, A_w_o, B_x, B_w1, B_w2, B_w3, B_w4, c, w_mod):
    del B_x
    hbm = pl.BlockSpec(memory_space=pltpu.HBM)
    out = pl.pallas_call(
        _kernel,
        grid=(1,),
        in_specs=[hbm, hbm, hbm, hbm, hbm, hbm, hbm, hbm, hbm, hbm,
                  pl.BlockSpec((1, M), lambda i: (0, 0)),
                  hbm],
        out_specs=hbm,
        out_shape=jax.ShapeDtypeStruct((S, M), bf16),
        scratch_shapes=[
            pltpu.VMEM((S, M), bf16),
            pltpu.VMEM((S, DC), bf16),
            pltpu.VMEM((S, M), bf16),
            pltpu.VMEM((M, 6 * M), bf16),
            pltpu.VMEM((8, 6 * M), f32),
            pltpu.VMEM((2, D, M), bf16),
            pltpu.VMEM((M, M), bf16),
            pltpu.VMEM((M, M), bf16),
            pltpu.VMEM((FP, M), bf16),
            pltpu.VMEM((FP, M), bf16),
            pltpu.VMEM((M, D), bf16),
            pltpu.VMEM((DC, D), bf16),
            pltpu.VMEM((DC, D), bf16),
            pltpu.VMEM((2, M, D), u32),
            pltpu.VMEM((2, DC, D), u32),
            pltpu.VMEM((2, DC, D), u32),
            pltpu.VMEM((S, D), bf16),
            pltpu.VMEM((S, D), bf16),
            pltpu.VMEM((S, D), bf16),
            pltpu.VMEM((S, M), f32),
            pltpu.VMEM((S, M), f32),
            pltpu.VMEM((S, M), f32),
            pltpu.VMEM((S + 16, M), f32),
            pltpu.VMEM((S, M), bf16),
            pltpu.SemaphoreType.DMA((7,)),
            pltpu.SemaphoreType.DMA((4, 2)),
            pltpu.SemaphoreType.DMA((2, S // PB)),
        ],
        compiler_params=pltpu.CompilerParams(
            dimension_semantics=("arbitrary",),
            vmem_limit_bytes=100 * 1024 * 1024,
            flags={"XLA_TPU_RESCHEDULE_DMA_DONES": True},
        ),
    )(A_x.reshape(S, M), A_c_kv.reshape(S, DC), A_w_q, A_w_uk, A_w_uv, A_w_o.reshape(H * D, M),
      B_w1, B_w2, B_w3.T, B_w4, c, w_mod)
    return out.reshape(1, S, M)
```

```python
import functools

import numpy as np
import jax
import jax.numpy as jnp
from jax import lax
import jax.experimental.pallas as pl
import jax.experimental.pallas.tpu as pltpu

S = 2048
M = 640
H = 32
D = 128
DC = 512
F = 1728
FP = 1792

BQ = 128
KC = 1024
PVC = 1024
QDELAY = 12
VDELAY = 8
PB = 256
SB = 128
RB = 512

LOG2E = 1.4426950408889634
QSCALE = float(D ** -0.5) * LOG2E
GELU_C = float(np.sqrt(2.0 / np.pi))
NEG = -1e30
NP = M // 128
NC = DC // 128
f32 = jnp.float32
bf16 = jnp.bfloat16
u32 = jnp.uint32


def _ln(x):
    m = jnp.mean(x, axis=-1, keepdims=True)
    xc = x - m
    v = jnp.mean(xc * xc, axis=-1, keepdims=True)
    return xc * lax.rsqrt(v + 1e-5)


def _gelu(x):
    u = x * (GELU_C + (GELU_C * 0.044715) * (x * x))
    hx = 0.5 * x
    return hx + hx * jnp.tanh(u)


def _dot(a, b):
    return jnp.dot(a, b, preferred_element_type=f32)


def _dot_nt(a, b):
    return lax.dot_general(a, b, (((1,), (1,)), ((), ())), preferred_element_type=f32)


def _kernel(x_hbm, ckv_hbm, wq_hbm, wuk_hbm, wuv_hbm, wo_hbm, w1_hbm, w2_hbm, w3t_hbm, w4_hbm, c_ref, wmod_hbm,
            out_hbm,
            x_s, ckv_s, hmod_s, wmod_s, mod_s, wo_s, w1_s, w2_s, w3t_s, w4_s,
            wq_s, wuk_s, wuv_s, rq_s, ruk_s, ruv_s,
            q_s, k_s, v_s, acc_s, x2_s, h_s, h1_s, out_s,
            sems, wsems, isems):
    wq_pairs = wq_hbm.bitcast(u32)
    wuk_pairs = wuk_hbm.bitcast(u32)
    wuv_pairs = wuv_hbm.bitcast(u32)

    def pcopies(j, sl):
        return [pltpu.make_async_copy(wq_pairs.at[:, j, :], rq_s.at[sl], wsems.at[0, sl]),
                pltpu.make_async_copy(wuk_pairs.at[:, j, :], ruk_s.at[sl], wsems.at[1, sl]),
                pltpu.make_async_copy(wuv_pairs.at[:, j, :], ruv_s.at[sl], wsems.at[2, sl])]

    def unpack_weights(sl, odd):
        for raw, dst in ((rq_s, wq_s), (ruk_s, wuk_s), (ruv_s, wuv_s)):
            bits = (raw[sl] & u32(0xFFFF0000)) if odd else (raw[sl] << u32(16))
            dst[...] = pltpu.bitcast(bits, f32).astype(bf16)

    def wocopy(j, sl):
        return pltpu.make_async_copy(wo_hbm.at[pl.ds(pl.multiple_of(j * 2 * D, 2 * D), 2 * D), :], wo_s.at[sl],
                                     wsems.at[3, sl])

    def in_copies(i):
        r = pl.ds(pl.multiple_of(i * PB, PB), PB)
        return [pltpu.make_async_copy(x_hbm.at[r, :], x_s.at[r, :], isems.at[0, i]),
                pltpu.make_async_copy(ckv_hbm.at[r, :], ckv_s.at[r, :], isems.at[1, i])]

    cp_wmod0 = pltpu.make_async_copy(wmod_hbm.at[:, 0:2 * M], wmod_s.at[:, 0:2 * M], sems.at[0])
    cp_wmod1 = pltpu.make_async_copy(wmod_hbm.at[:, 2 * M:6 * M], wmod_s.at[:, 2 * M:6 * M], sems.at[1])
    cp_w1 = pltpu.make_async_copy(w1_hbm, w1_s, sems.at[2])
    cp_w2 = pltpu.make_async_copy(w2_hbm, w2_s, sems.at[3])
    cp_w3 = pltpu.make_async_copy(w3t_hbm, w3t_s.at[0:F, :], sems.at[4])
    cp_w4 = pltpu.make_async_copy(w4_hbm, w4_s.at[0:F, :], sems.at[5])
    cp_out = pltpu.make_async_copy(out_s, out_hbm, sems.at[6])

    def proj(src_s, w_ref, nt, rs):
        acc = None
        for t in range(nt):
            o = _dot(src_s[rs, t * 128:(t + 1) * 128], w_ref[t * 128:(t + 1) * 128, :])
            acc = o if acc is None else acc + o
        return acc

    def kpiece(rs):
        k_s[rs, :] = proj(ckv_s, wuk_s, NC, rs).astype(bf16)

    def vpiece(rs):
        v_s[rs, :] = proj(ckv_s, wuv_s, NC, rs).astype(bf16)

    def qpiece(rs):
        q_s[rs, :] = (proj(hmod_s, wq_s, NP, rs) * QSCALE).astype(bf16)

    nb = S // PB
    LOOK = 2
    cp_wmod0.start()
    for cp in pcopies(0, 0):
        cp.start()
    for i in range(LOOK):
        for cp in in_copies(i):
            cp.start()
    acc_s[...] = jnp.zeros((S, M), f32)
    h1_s[0:8, :] = jnp.zeros((8, M), f32)
    h1_s[S + 8:S + 16, :] = jnp.zeros((8, M), f32)
    w3t_s[F:FP, :] = jnp.zeros((FP - F, M), bf16)
    w4_s[F:FP, :] = jnp.zeros((FP - F, M), bf16)

    c = c_ref[...].astype(f32)
    sc = c * (1.0 / (1.0 + jnp.exp(-c)))
    sc16 = jnp.broadcast_to(sc, (16, M)).astype(bf16)
    cp_wmod0.wait()
    mod_s[:, 0:2 * M] = _dot(sc16, wmod_s[:, 0:2 * M])[0:8, :]
    sa = mod_s[0:1, 0:M]
    ca = mod_s[0:1, M:2 * M]
    for cp in pcopies(0, 0):
        cp.wait()
    unpack_weights(0, odd=False)

    def first_body(i, carry, do_v, do_q):
        r = pl.ds(pl.multiple_of(i * PB, PB), PB)
        for cp in in_copies(i):
            cp.wait()

        @pl.when(i + LOOK < nb)
        def _():
            for cp in in_copies(i + LOOK):
                cp.start()

        @pl.when(i + LOOK == nb)
        def _():
            wocopy(0, 0).start()
            for cp in pcopies(1, 1):
                cp.start()

        kpiece(r)
        if do_v:
            vpiece(r)
        hmod_s[r, :] = (_ln(x_s[r, :].astype(f32)) * (1.0 + ca) + sa).astype(bf16)
        if do_q:
            qpiece(r)
        return carry

    nv, nqd = VDELAY * BQ // PB, QDELAY * BQ // PB
    lax.fori_loop(0, nv, functools.partial(first_body, do_v=False, do_q=False), 0)
    lax.fori_loop(nv, nqd, functools.partial(first_body, do_v=True, do_q=False), 0)
    lax.fori_loop(nqd, nb, functools.partial(first_body, do_v=True, do_q=True), 0)
    cp_wmod1.start()
    cp_w1.start()
    cp_w2.start()
    cp_w3.start()
    cp_w4.start()

    nq = S // BQ

    def head_body(gs, odd, next_slot):
        row = lax.broadcasted_iota(jnp.int32, (128, 128), 0)
        col = lax.broadcasted_iota(jnp.int32, (128, 128), 1)
        causal = col <= row

        def blk(i):
            return slice(i * BQ, i * BQ + BQ)

        def chunks(i, cwmax):
            n = (i + 1) * BQ
            return [(c0, min(cwmax, n - c0)) for c0 in range(0, n, cwmax)]

        def qk_tiles(i, c0, cw):
            s = _dot_nt(q_s[blk(i), :], k_s[c0:c0 + cw, :])
            tiles = []
            for t in range(cw // 128):
                st = s[:, t * 128:(t + 1) * 128]
                if c0 + t * 128 == i * BQ:
                    st = jnp.where(causal, st, NEG)
                tiles.append(st)
            return tiles

        def rowmax(tiles):
            m = tiles[0]
            for st in tiles[1:]:
                m = jnp.maximum(m, st)
            return jnp.broadcast_to(jnp.max(m, axis=-1, keepdims=True), (BQ, 128))

        pending = []
        for i in range(VDELAY - 1, -1, -1):
            vpiece(blk(i))
        cur = []
        for (c0, cw) in chunks(nq - 1, KC):
            cur += qk_tiles(nq - 1, c0, cw)
        for i in range(QDELAY - 1, -1, -1):
            qpiece(blk(i))
        unpack_weights(next_slot, odd=not odd)
        mb = rowmax(cur)

        for i in range(nq - 1, -1, -1):
            nxt_chunks = chunks(i - 1, KC) if i > 0 else []
            nxt = []
            l = None
            acc = None
            prev_o = None
            ci = 0
            pv_chunks = chunks(i, PVC)
            npv = len(pv_chunks)
            for pi, (c0, cw) in enumerate(pv_chunks):
                mbc = mb if prev_o is None else mb + prev_o * 0.0
                ps = [jnp.exp2(cur[t] - mbc) for t in range(c0 // 128, (c0 + cw) // 128)]
                pj = ps[0] if len(ps) == 1 else jnp.concatenate(ps, axis=1)
                psum = ps[0]
                for p in ps[1:]:
                    psum = psum + p
                l = psum if l is None else l + psum
                o = _dot(pj.astype(bf16), v_s[c0:c0 + cw, :])
                prev_o = o
                acc = o if acc is None else acc + o
                while ci < len(nxt_chunks) and ci * npv < (pi + 1) * len(nxt_chunks):
                    nxt += qk_tiles(i - 1, *nxt_chunks[ci])
                    ci += 1
                for _ in range(-(-len(pending) // (npv - pi))):
                    pending.pop(0)()
            l = jnp.sum(l, axis=-1, keepdims=True)
            r = pl.reciprocal(l, approx=True)
            r = r * (2.0 - l * r)
            ctx = (acc * r).astype(bf16)
            acc_s[blk(i), :] = acc_s[blk(i), :] + _dot(ctx, wo_s[gs, (D if odd else 0):(2 * D if odd else D), :])
            pending.append(lambda i=i: kpiece(blk(i)))
            if i >= QDELAY:
                pending.append(lambda i=i: qpiece(blk(i)))
            if i >= VDELAY:
                pending.append(lambda i=i: vpiece(blk(i)))
            if nxt:
                cur = nxt
                mb = rowmax(cur)
        while pending:
            pending.pop(0)()

    G = H // 2

    def two_heads(g, carry):
        gs = g % 2
        wocopy(g, gs).wait()
        wocopy(jnp.minimum(g + 1, G - 1), 1 - gs).start()
        head_body(gs, False, gs)
        for cp in pcopies(jnp.minimum(g + 1, G - 1), 1 - gs):
            cp.wait()
        for cp in pcopies(jnp.minimum(g + 2, G - 1), gs):
            cp.start()
        head_body(gs, True, 1 - gs)
        return carry

    lax.fori_loop(0, G, two_heads, 0)
    wocopy(G - 1, G % 2).wait()
    for cp in pcopies(G - 1, (G - 1) % 2):
        cp.wait()

    cp_wmod1.wait()
    mod_s[:, 2 * M:6 * M] = _dot(sc16, wmod_s[:, 2 * M:6 * M])[0:8, :]
    cp_w1.wait()
    cp_w2.wait()
    cp_w3.wait()
    cp_w4.wait()
    ga = mod_s[0:1, 2 * M:3 * M]
    sb = mod_s[0:1, 3 * M:4 * M]
    cb = mod_s[0:1, 4 * M:5 * M]
    gb = mod_s[0:1, 5 * M:6 * M]

    for k in range(S // SB):
        r = slice(k * SB, (k + 1) * SB)
        x2 = x_s[r, :].astype(f32) + ga * acc_s[r, :]
        x2_s[r, :] = x2
        hb = _ln(x2) * (1.0 + cb) + sb
        h_s[r, :] = hb
        h1_s[k * SB + 8:(k + 1) * SB + 8, :] = _gelu(_dot(_ln(hb).astype(bf16), w1_s[...]))

    lane = lax.broadcasted_iota(jnp.int32, (SB, 128), 1)

    def mix(r0):
        r = pl.ds(r0, SB)
        win = h1_s[pl.ds(r0, SB + 16), :]

        def sh(off, t):
            return win[8 + off:8 + off + SB, t * 128:(t + 1) * 128]

        t0 = sh(-1, 0)
        t1 = jnp.where(lane < 32, sh(-1, 1), sh(1, 1))
        t2 = jnp.where(lane < 64, sh(1, 2), sh(-2, 2))
        t3 = jnp.where(lane < 96, sh(-2, 3), sh(2, 3))
        t4 = sh(2, 4)
        g = jnp.concatenate([t0, t1, t2, t3, t4], axis=1).astype(bf16)
        x1 = h_s[r, :] + _dot(g, w2_s[...])
        y = x2_s[r, :] + gb * x1
        return y, _ln(x1).astype(bf16)

    def mlp(r0, y, ln1):
        r = pl.ds(r0, SB)
        u = _gelu(_dot_nt(ln1, w3t_s[...])).astype(bf16)
        out_s[r, :] = (y + gb * _dot(u, w4_s[...])).astype(bf16)
        pltpu.make_async_copy(out_s.at[r, :], out_hbm.at[r, :], sems.at[6]).start()

    def pass2(i, carry):
        base = pl.multiple_of(i * RB, RB)
        starts = [pl.multiple_of(base + k * SB, SB) for k in range(RB // SB)]
        staged = [mix(r0) for r0 in starts]
        for r0, (y, ln1) in zip(starts, staged):
            mlp(r0, y, ln1)
        return carry

    lax.fori_loop(0, S // RB, pass2, 0)
    cp_out.wait()


@jax.jit
def pallas_adaLN_cond__compressed_kv_cla__mixer_s_mlp__prompt_kernel(
        A_x, A_c_kv, A_w_q, A_w_uk, A_w_uv, A_w_o, B_x, B_w1, B_w2, B_w3, B_w4, c, w_mod):
    del B_x
    hbm = pl.BlockSpec(memory_space=pltpu.HBM)
    out = pl.pallas_call(
        _kernel,
        grid=(1,),
        in_specs=[hbm, hbm, hbm, hbm, hbm, hbm, hbm, hbm, hbm, hbm,
                  pl.BlockSpec((1, M), lambda i: (0, 0)),
                  hbm],
        out_specs=hbm,
        out_shape=jax.ShapeDtypeStruct((S, M), bf16),
        scratch_shapes=[
            pltpu.VMEM((S, M), bf16),
            pltpu.VMEM((S, DC), bf16),
            pltpu.VMEM((S, M), bf16),
            pltpu.VMEM((M, 6 * M), bf16),
            pltpu.VMEM((8, 6 * M), f32),
            pltpu.VMEM((2, 2 * D, M), bf16),
            pltpu.VMEM((M, M), bf16),
            pltpu.VMEM((M, M), bf16),
            pltpu.VMEM((FP, M), bf16),
            pltpu.VMEM((FP, M), bf16),
            pltpu.VMEM((M, D), bf16),
            pltpu.VMEM((DC, D), bf16),
            pltpu.VMEM((DC, D), bf16),
            pltpu.VMEM((2, M, D), u32),
            pltpu.VMEM((2, DC, D), u32),
            pltpu.VMEM((2, DC, D), u32),
            pltpu.VMEM((S, D), bf16),
            pltpu.VMEM((S, D), bf16),
            pltpu.VMEM((S, D), bf16),
            pltpu.VMEM((S, M), f32),
            pltpu.VMEM((S, M), f32),
            pltpu.VMEM((S, M), f32),
            pltpu.VMEM((S + 16, M), f32),
            pltpu.VMEM((S, M), bf16),
            pltpu.SemaphoreType.DMA((7,)),
            pltpu.SemaphoreType.DMA((4, 2)),
            pltpu.SemaphoreType.DMA((2, S // PB)),
        ],
        compiler_params=pltpu.CompilerParams(
            dimension_semantics=("arbitrary",),
            vmem_limit_bytes=100 * 1024 * 1024,
            flags={"XLA_TPU_RESCHEDULE_DMA_DONES": True},
        ),
    )(A_x.reshape(S, M), A_c_kv.reshape(S, DC), A_w_q, A_w_uk, A_w_uv, A_w_o.reshape(H * D, M),
      B_w1, B_w2, B_w3.T, B_w4, c, w_mod)
    return out.reshape(1, S, M)
```

```python
import functools

import numpy as np
import jax
import jax.numpy as jnp
from jax import lax
import jax.experimental.pallas as pl
import jax.experimental.pallas.tpu as pltpu

S = 2048
M = 640
H = 32
D = 128
DC = 512
F = 1728
FP = 1792

BQ = 128
KC = 1024
PVC = 1024
QDELAY = 12
VDELAY = 8
PB = 256
SB = 128
RB = 512

LOG2E = 1.4426950408889634
QSCALE = float(D ** -0.5) * LOG2E
GELU_C = float(np.sqrt(2.0 / np.pi))
NEG = -1e30
NP = M // 128
NC = DC // 128
f32 = jnp.float32
bf16 = jnp.bfloat16
u32 = jnp.uint32


def _ln(x):
    m = jnp.mean(x, axis=-1, keepdims=True)
    xc = x - m
    v = jnp.mean(xc * xc, axis=-1, keepdims=True)
    return xc * lax.rsqrt(v + 1e-5)


def _gelu(x):
    u = x * (GELU_C + (GELU_C * 0.044715) * (x * x))
    hx = 0.5 * x
    return hx + hx * jnp.tanh(u)


def _dot(a, b):
    return jnp.dot(a, b, preferred_element_type=f32)


def _dot_nt(a, b):
    return lax.dot_general(a, b, (((1,), (1,)), ((), ())), preferred_element_type=f32)


def _kernel(x_hbm, ckv_hbm, wq_hbm, wuk_hbm, wuv_hbm, wo_hbm, w1_hbm, w2_hbm, w3t_hbm, w4_hbm, c_hbm, wmod_hbm,
            out_hbm,
            x_s, ckv_s, c_s, hmod_s, wmod_s, mod_s, wo_s, w1_s, w2_s, w3t_s, w4_s,
            wq_s, wuk_s, wuv_s, rq_s, ruk_s, ruv_s,
            q_s, k_s, v_s, acc_s, x2_s, h_s, h1_s, out_s,
            sems, wsems, isems):
    wq_pairs = wq_hbm.bitcast(u32)
    wuk_pairs = wuk_hbm.bitcast(u32)
    wuv_pairs = wuv_hbm.bitcast(u32)

    def pcopies(j, sl):
        return [pltpu.make_async_copy(wq_pairs.at[:, j, :], rq_s.at[sl], wsems.at[0, sl]),
                pltpu.make_async_copy(wuk_pairs.at[:, j, :], ruk_s.at[sl], wsems.at[1, sl]),
                pltpu.make_async_copy(wuv_pairs.at[:, j, :], ruv_s.at[sl], wsems.at[2, sl])]

    def unpack_weights(sl, odd):
        for raw, dst in ((rq_s, wq_s), (ruk_s, wuk_s), (ruv_s, wuv_s)):
            bits = (raw[sl] & u32(0xFFFF0000)) if odd else (raw[sl] << u32(16))
            dst[...] = pltpu.bitcast(bits, f32).astype(bf16)

    def wocopy(j, sl):
        return pltpu.make_async_copy(wo_hbm.at[pl.ds(pl.multiple_of(j * 2 * D, 2 * D), 2 * D), :], wo_s.at[sl],
                                     wsems.at[3, sl])

    def in_copies(i):
        r = pl.ds(pl.multiple_of(i * PB, PB), PB)
        return [pltpu.make_async_copy(x_hbm.at[r, :], x_s.at[r, :], isems.at[0, i]),
                pltpu.make_async_copy(ckv_hbm.at[r, :], ckv_s.at[r, :], isems.at[1, i])]

    cp_c = pltpu.make_async_copy(c_hbm, c_s, sems.at[7])
    cp_wmod0 = pltpu.make_async_copy(wmod_hbm.at[:, 0:2 * M], wmod_s.at[:, 0:2 * M], sems.at[0])
    cp_wmod1 = pltpu.make_async_copy(wmod_hbm.at[:, 2 * M:6 * M], wmod_s.at[:, 2 * M:6 * M], sems.at[1])
    cp_w1 = pltpu.make_async_copy(w1_hbm, w1_s, sems.at[2])
    cp_w2 = pltpu.make_async_copy(w2_hbm, w2_s, sems.at[3])
    cp_w3 = pltpu.make_async_copy(w3t_hbm, w3t_s.at[0:F, :], sems.at[4])
    cp_w4 = pltpu.make_async_copy(w4_hbm, w4_s.at[0:F, :], sems.at[5])
    cp_out = pltpu.make_async_copy(out_s, out_hbm, sems.at[6])

    def proj(src_s, w_ref, nt, rs):
        acc = None
        for t in range(nt):
            o = _dot(src_s[rs, t * 128:(t + 1) * 128], w_ref[t * 128:(t + 1) * 128, :])
            acc = o if acc is None else acc + o
        return acc

    def kpiece(rs):
        k_s[rs, :] = proj(ckv_s, wuk_s, NC, rs).astype(bf16)

    def vpiece(rs):
        v_s[rs, :] = proj(ckv_s, wuv_s, NC, rs).astype(bf16)

    def qpiece(rs):
        q_s[rs, :] = (proj(hmod_s, wq_s, NP, rs) * QSCALE).astype(bf16)

    nb = S // PB
    LOOK = 2
    cp_c.start()
    cp_wmod0.start()
    for cp in pcopies(0, 0):
        cp.start()
    for j in range(LOOK):
        for cp in in_copies(nb - 1 - j):
            cp.start()
    acc_s[...] = jnp.zeros((S, M), f32)
    h1_s[0:8, :] = jnp.zeros((8, M), f32)
    h1_s[S + 8:S + 16, :] = jnp.zeros((8, M), f32)
    w3t_s[F:FP, :] = jnp.zeros((FP - F, M), bf16)
    w4_s[F:FP, :] = jnp.zeros((FP - F, M), bf16)

    cp_c.wait()
    c = c_s[...].astype(f32)
    sc = c * (1.0 / (1.0 + jnp.exp(-c)))
    sc16 = jnp.broadcast_to(sc, (16, M)).astype(bf16)
    cp_wmod0.wait()
    mod_s[:, 0:2 * M] = _dot(sc16, wmod_s[:, 0:2 * M])[0:8, :]
    sa = mod_s[0:1, 0:M]
    ca = mod_s[0:1, M:2 * M]
    for cp in pcopies(0, 0):
        cp.wait()
    unpack_weights(0, odd=False)

    def first_body(j, carry, do_v, do_q):
        i = nb - 1 - j
        r = pl.ds(pl.multiple_of(i * PB, PB), PB)
        for cp in in_copies(i):
            cp.wait()

        @pl.when(j + LOOK < nb)
        def _():
            for cp in in_copies(i - LOOK):
                cp.start()

        @pl.when(j + LOOK == nb)
        def _():
            wocopy(0, 0).start()

        kpiece(r)
        if do_v:
            vpiece(r)
        hmod_s[r, :] = (_ln(x_s[r, :].astype(f32)) * (1.0 + ca) + sa).astype(bf16)
        if do_q:
            qpiece(r)
        return carry

    nv, nqd = VDELAY * BQ // PB, QDELAY * BQ // PB
    lax.fori_loop(0, nb - nqd, functools.partial(first_body, do_v=True, do_q=True), 0)
    lax.fori_loop(nb - nqd, nb - nv, functools.partial(first_body, do_v=True, do_q=False), 0)
    lax.fori_loop(nb - nv, nb, functools.partial(first_body, do_v=False, do_q=False), 0)
    for cp in pcopies(1, 1):
        cp.start()
    cp_wmod1.start()
    cp_w1.start()
    cp_w2.start()
    cp_w3.start()
    cp_w4.start()

    nq = S // BQ

    def head_body(gs, odd, next_slot):
        row = lax.broadcasted_iota(jnp.int32, (128, 128), 0)
        col = lax.broadcasted_iota(jnp.int32, (128, 128), 1)
        causal = col <= row

        def blk(i):
            return slice(i * BQ, i * BQ + BQ)

        def chunks(i, cwmax):
            n = (i + 1) * BQ
            return [(c0, min(cwmax, n - c0)) for c0 in range(0, n, cwmax)]

        def qk_tiles(i, c0, cw):
            s = _dot_nt(q_s[blk(i), :], k_s[c0:c0 + cw, :])
            tiles = []
            for t in range(cw // 128):
                st = s[:, t * 128:(t + 1) * 128]
                if c0 + t * 128 == i * BQ:
                    st = jnp.where(causal, st, NEG)
                tiles.append(st)
            return tiles

        def rowmax(tiles):
            m = tiles[0]
            for st in tiles[1:]:
                m = jnp.maximum(m, st)
            return jnp.broadcast_to(jnp.max(m, axis=-1, keepdims=True), (BQ, 128))

        pending = []
        for i in range(VDELAY - 1, -1, -1):
            vpiece(blk(i))
        cur = []
        for (c0, cw) in chunks(nq - 1, KC):
            cur += qk_tiles(nq - 1, c0, cw)
        for i in range(QDELAY - 1, -1, -1):
            qpiece(blk(i))
        unpack_weights(next_slot, odd=not odd)
        mb = rowmax(cur)

        for i in range(nq - 1, -1, -1):
            nxt_chunks = chunks(i - 1, KC) if i > 0 else []
            nxt = []
            l = None
            acc = None
            prev_o = None
            ci = 0
            pv_chunks = chunks(i, PVC)
            npv = len(pv_chunks)
            for pi, (c0, cw) in enumerate(pv_chunks):
                mbc = mb if prev_o is None else mb + prev_o * 0.0
                ps = [jnp.exp2(cur[t] - mbc) for t in range(c0 // 128, (c0 + cw) // 128)]
                pj = ps[0] if len(ps) == 1 else jnp.concatenate(ps, axis=1)
                psum = ps[0]
                for p in ps[1:]:
                    psum = psum + p
                l = psum if l is None else l + psum
                o = _dot(pj.astype(bf16), v_s[c0:c0 + cw, :])
                prev_o = o
                acc = o if acc is None else acc + o
                while ci < len(nxt_chunks) and ci * npv < (pi + 1) * len(nxt_chunks):
                    nxt += qk_tiles(i - 1, *nxt_chunks[ci])
                    ci += 1
                for _ in range(-(-len(pending) // (npv - pi))):
                    pending.pop(0)()
            l = jnp.sum(l, axis=-1, keepdims=True)
            r = pl.reciprocal(l, approx=True)
            r = r * (2.0 - l * r)
            ctx = (acc * r).astype(bf16)
            acc_s[blk(i), :] = acc_s[blk(i), :] + _dot(ctx, wo_s[gs, (D if odd else 0):(2 * D if odd else D), :])
            pending.append(lambda i=i: kpiece(blk(i)))
            if i >= QDELAY:
                pending.append(lambda i=i: qpiece(blk(i)))
            if i >= VDELAY:
                pending.append(lambda i=i: vpiece(blk(i)))
            if nxt:
                cur = nxt
                mb = rowmax(cur)
        while pending:
            pending.pop(0)()

    G = H // 2

    def two_heads(g, carry):
        gs = g % 2
        wocopy(g, gs).wait()
        wocopy(jnp.minimum(g + 1, G - 1), 1 - gs).start()
        head_body(gs, False, gs)
        for cp in pcopies(jnp.minimum(g + 1, G - 1), 1 - gs):
            cp.wait()
        for cp in pcopies(jnp.minimum(g + 2, G - 1), gs):
            cp.start()
        head_body(gs, True, 1 - gs)
        return carry

    lax.fori_loop(0, G, two_heads, 0)
    wocopy(G - 1, G % 2).wait()
    for cp in pcopies(G - 1, (G - 1) % 2):
        cp.wait()

    cp_wmod1.wait()
    mod_s[:, 2 * M:6 * M] = _dot(sc16, wmod_s[:, 2 * M:6 * M])[0:8, :]
    cp_w1.wait()
    cp_w2.wait()
    cp_w3.wait()
    cp_w4.wait()
    ga = mod_s[0:1, 2 * M:3 * M]
    sb = mod_s[0:1, 3 * M:4 * M]
    cb = mod_s[0:1, 4 * M:5 * M]
    gb = mod_s[0:1, 5 * M:6 * M]

    for k in range(S // SB):
        r = slice(k * SB, (k + 1) * SB)
        x2 = x_s[r, :].astype(f32) + ga * acc_s[r, :]
        x2_s[r, :] = x2
        hb = _ln(x2) * (1.0 + cb) + sb
        h_s[r, :] = hb
        h1_s[k * SB + 8:(k + 1) * SB + 8, :] = _gelu(_dot(_ln(hb).astype(bf16), w1_s[...]))

    lane = lax.broadcasted_iota(jnp.int32, (SB, 128), 1)

    def mix(r0):
        r = pl.ds(r0, SB)
        win = h1_s[pl.ds(r0, SB + 16), :]

        def sh(off, t):
            return win[8 + off:8 + off + SB, t * 128:(t + 1) * 128]

        t0 = sh(-1, 0)
        t1 = jnp.where(lane < 32, sh(-1, 1), sh(1, 1))
        t2 = jnp.where(lane < 64, sh(1, 2), sh(-2, 2))
        t3 = jnp.where(lane < 96, sh(-2, 3), sh(2, 3))
        t4 = sh(2, 4)
        g = jnp.concatenate([t0, t1, t2, t3, t4], axis=1).astype(bf16)
        x1 = h_s[r, :] + _dot(g, w2_s[...])
        y = x2_s[r, :] + gb * x1
        return y, _ln(x1).astype(bf16)

    def mlp(r0, y, ln1):
        r = pl.ds(r0, SB)
        u = _gelu(_dot_nt(ln1, w3t_s[...])).astype(bf16)
        out_s[r, :] = (y + gb * _dot(u, w4_s[...])).astype(bf16)
        pltpu.make_async_copy(out_s.at[r, :], out_hbm.at[r, :], sems.at[6]).start()

    def pass2(i, carry):
        base = pl.multiple_of(i * RB, RB)
        starts = [pl.multiple_of(base + k * SB, SB) for k in range(RB // SB)]
        staged = [mix(r0) for r0 in starts]
        for r0, (y, ln1) in zip(starts, staged):
            mlp(r0, y, ln1)
        return carry

    lax.fori_loop(0, S // RB, pass2, 0)
    cp_out.wait()


@jax.jit
def pallas_adaLN_cond__compressed_kv_cla__mixer_s_mlp__prompt_kernel(
        A_x, A_c_kv, A_w_q, A_w_uk, A_w_uv, A_w_o, B_x, B_w1, B_w2, B_w3, B_w4, c, w_mod):
    del B_x
    hbm = pl.BlockSpec(memory_space=pltpu.HBM)
    out = pl.pallas_call(
        _kernel,
        in_specs=[hbm] * 12,
        out_specs=hbm,
        out_shape=jax.ShapeDtypeStruct((S, M), bf16),
        scratch_shapes=[
            pltpu.VMEM((S, M), bf16),
            pltpu.VMEM((S, DC), bf16),
            pltpu.VMEM((1, M), bf16),
            pltpu.VMEM((S, M), bf16),
            pltpu.VMEM((M, 6 * M), bf16),
            pltpu.VMEM((8, 6 * M), f32),
            pltpu.VMEM((2, 2 * D, M), bf16),
            pltpu.VMEM((M, M), bf16),
            pltpu.VMEM((M, M), bf16),
            pltpu.VMEM((FP, M), bf16),
            pltpu.VMEM((FP, M), bf16),
            pltpu.VMEM((M, D), bf16),
            pltpu.VMEM((DC, D), bf16),
            pltpu.VMEM((DC, D), bf16),
            pltpu.VMEM((2, M, D), u32),
            pltpu.VMEM((2, DC, D), u32),
            pltpu.VMEM((2, DC, D), u32),
            pltpu.VMEM((S, D), bf16),
            pltpu.VMEM((S, D), bf16),
            pltpu.VMEM((S, D), bf16),
            pltpu.VMEM((S, M), f32),
            pltpu.VMEM((S, M), f32),
            pltpu.VMEM((S, M), f32),
            pltpu.VMEM((S + 16, M), f32),
            pltpu.VMEM((S, M), bf16),
            pltpu.SemaphoreType.DMA((8,)),
            pltpu.SemaphoreType.DMA((4, 2)),
            pltpu.SemaphoreType.DMA((2, S // PB)),
        ],
        compiler_params=pltpu.CompilerParams(
            vmem_limit_bytes=100 * 1024 * 1024,
            flags={"XLA_TPU_RESCHEDULE_DMA_DONES": True},
        ),
    )(A_x.reshape(S, M), A_c_kv.reshape(S, DC), A_w_q, A_w_uk, A_w_uv, A_w_o.reshape(H * D, M),
      B_w1, B_w2, B_w3.T, B_w4, c, w_mod)
    return out.reshape(1, S, M)
```

```python
import functools

import numpy as np
import jax
import jax.numpy as jnp
from jax import lax
import jax.experimental.pallas as pl
import jax.experimental.pallas.tpu as pltpu

S = 2048
M = 640
H = 32
D = 128
DC = 512
F = 1728
FP = 1792

BQ = 128
KC = 1024
PVC = 1024
QDELAY = 12
VDELAY = 8
PB = 256
SB = 128
RB = 512

LOG2E = 1.4426950408889634
QSCALE = float(D ** -0.5) * LOG2E
GELU_C = float(np.sqrt(2.0 / np.pi))
NEG = -1e30
NP = M // 128
NC = DC // 128
f32 = jnp.float32
bf16 = jnp.bfloat16
u32 = jnp.uint32


def _ln(x):
    m = jnp.mean(x, axis=-1, keepdims=True)
    xc = x - m
    v = jnp.mean(xc * xc, axis=-1, keepdims=True)
    return xc * lax.rsqrt(v + 1e-5)


def _gelu(x):
    u = x * (GELU_C + (GELU_C * 0.044715) * (x * x))
    hx = 0.5 * x
    return hx + hx * jnp.tanh(u)


def _dot(a, b):
    return jnp.dot(a, b, preferred_element_type=f32)


def _dot_nt(a, b):
    return lax.dot_general(a, b, (((1,), (1,)), ((), ())), preferred_element_type=f32)


def _kernel(x_hbm, ckv_hbm, wq_hbm, wuk_hbm, wuv_hbm, wo_hbm, w1_hbm, w2_hbm, w3t_hbm, w4_hbm, c_hbm, wmod_hbm,
            out_hbm,
            x_s, ckv_s, c_s, hmod_s, wmod_s, wo_s, w1_s, w2_s, w3t_s, w4_s,
            wq_s, wuk_s, wuv_s, rq_s, ruk_s, ruv_s,
            q_s, k_s, v_s, acc_s, x2_s, h_s, h1_s, out_s,
            sems, wsems, isems):
    wq_pairs = wq_hbm.bitcast(u32)
    wuk_pairs = wuk_hbm.bitcast(u32)
    wuv_pairs = wuv_hbm.bitcast(u32)

    def pcopies(j, sl):
        return [pltpu.make_async_copy(wq_pairs.at[:, j, :], rq_s.at[sl], wsems.at[0, sl]),
                pltpu.make_async_copy(wuk_pairs.at[:, j, :], ruk_s.at[sl], wsems.at[1, sl]),
                pltpu.make_async_copy(wuv_pairs.at[:, j, :], ruv_s.at[sl], wsems.at[2, sl])]

    def unpack_weights(sl, odd):
        for raw, dst in ((rq_s, wq_s), (ruk_s, wuk_s), (ruv_s, wuv_s)):
            bits = (raw[sl] & u32(0xFFFF0000)) if odd else (raw[sl] << u32(16))
            dst[...] = pltpu.bitcast(bits, f32).astype(bf16)

    def wocopy(j, sl):
        return pltpu.make_async_copy(wo_hbm.at[pl.ds(pl.multiple_of(j * 2 * D, 2 * D), 2 * D), :], wo_s.at[sl],
                                     wsems.at[3, sl])

    def in_copies(i):
        r = pl.ds(pl.multiple_of(i * PB, PB), PB)
        return [pltpu.make_async_copy(x_hbm.at[r, :], x_s.at[r, :], isems.at[0, i]),
                pltpu.make_async_copy(ckv_hbm.at[r, :], ckv_s.at[r, :], isems.at[1, i])]

    cp_c = pltpu.make_async_copy(c_hbm, c_s, sems.at[7])
    cp_wmod0 = pltpu.make_async_copy(wmod_hbm.at[:, 0:2 * M], wmod_s.at[:, 0:2 * M], sems.at[0])
    cp_wmod1 = pltpu.make_async_copy(wmod_hbm.at[:, 2 * M:6 * M], wmod_s.at[:, 2 * M:6 * M], sems.at[1])
    cp_w1 = pltpu.make_async_copy(w1_hbm, w1_s, sems.at[2])
    cp_w2 = pltpu.make_async_copy(w2_hbm, w2_s, sems.at[3])
    cp_w3 = pltpu.make_async_copy(w3t_hbm, w3t_s.at[0:F, :], sems.at[4])
    cp_w4 = pltpu.make_async_copy(w4_hbm, w4_s.at[0:F, :], sems.at[5])
    cp_out = pltpu.make_async_copy(out_s, out_hbm, sems.at[6])

    def proj(src_s, w_ref, nt, rs):
        acc = None
        for t in range(nt):
            o = _dot(src_s[rs, t * 128:(t + 1) * 128], w_ref[t * 128:(t + 1) * 128, :])
            acc = o if acc is None else acc + o
        return acc

    def kpiece(rs):
        k_s[rs, :] = proj(ckv_s, wuk_s, NC, rs).astype(bf16)

    def vpiece(rs):
        v_s[rs, :] = proj(ckv_s, wuv_s, NC, rs).astype(bf16)

    def qpiece(rs):
        q_s[rs, :] = (proj(hmod_s, wq_s, NP, rs) * QSCALE).astype(bf16)

    nb = S // PB
    LOOK = 2
    cp_c.start()
    cp_wmod0.start()
    for cp in pcopies(0, 0):
        cp.start()
    for j in range(LOOK):
        for cp in in_copies(nb - 1 - j):
            cp.start()
    acc_s[...] = jnp.zeros((S, M), f32)
    h1_s[0:8, :] = jnp.zeros((8, M), f32)
    h1_s[S + 8:S + 16, :] = jnp.zeros((8, M), f32)
    w3t_s[F:FP, :] = jnp.zeros((FP - F, M), bf16)
    w4_s[F:FP, :] = jnp.zeros((FP - F, M), bf16)

    cp_c.wait()
    c = c_s[...].astype(f32)
    sc = c * (1.0 / (1.0 + jnp.exp(-c)))
    sc16 = jnp.broadcast_to(sc, (16, M)).astype(bf16)
    cp_wmod0.wait()
    sa, ca = (_dot(sc16, wmod_s[:, j * M:(j + 1) * M])[0:1, :] for j in range(2))
    for cp in pcopies(0, 0):
        cp.wait()
    unpack_weights(0, odd=False)

    def first_body(j, carry, do_v, do_q):
        i = nb - 1 - j
        r = pl.ds(pl.multiple_of(i * PB, PB), PB)
        for cp in in_copies(i):
            cp.wait()

        @pl.when(j + LOOK < nb)
        def _():
            for cp in in_copies(i - LOOK):
                cp.start()

        @pl.when(j + LOOK == nb)
        def _():
            wocopy(0, 0).start()

        kpiece(r)
        if do_v:
            vpiece(r)
        hmod_s[r, :] = (_ln(x_s[r, :].astype(f32)) * (1.0 + ca) + sa).astype(bf16)
        if do_q:
            qpiece(r)
        return carry

    nv, nqd = VDELAY * BQ // PB, QDELAY * BQ // PB
    lax.fori_loop(0, nb - nqd, functools.partial(first_body, do_v=True, do_q=True), 0)
    lax.fori_loop(nb - nqd, nb - nv, functools.partial(first_body, do_v=True, do_q=False), 0)
    lax.fori_loop(nb - nv, nb, functools.partial(first_body, do_v=False, do_q=False), 0)
    for cp in pcopies(1, 1):
        cp.start()
    cp_wmod1.start()
    cp_w1.start()
    cp_w2.start()
    cp_w3.start()
    cp_w4.start()

    nq = S // BQ

    def head_body(gs, odd, next_slot):
        row = lax.broadcasted_iota(jnp.int32, (128, 128), 0)
        col = lax.broadcasted_iota(jnp.int32, (128, 128), 1)
        causal = col <= row

        def blk(i):
            return slice(i * BQ, i * BQ + BQ)

        def chunks(i, cwmax):
            n = (i + 1) * BQ
            return [(c0, min(cwmax, n - c0)) for c0 in range(0, n, cwmax)]

        def qk_tiles(i, c0, cw):
            s = _dot_nt(q_s[blk(i), :], k_s[c0:c0 + cw, :])
            tiles = []
            for t in range(cw // 128):
                st = s[:, t * 128:(t + 1) * 128]
                if c0 + t * 128 == i * BQ:
                    st = jnp.where(causal, st, NEG)
                tiles.append(st)
            return tiles

        def rowmax(tiles):
            m = tiles[0]
            for st in tiles[1:]:
                m = jnp.maximum(m, st)
            return jnp.broadcast_to(jnp.max(m, axis=-1, keepdims=True), (BQ, 128))

        pending = []
        for i in range(VDELAY - 1, -1, -1):
            vpiece(blk(i))
        cur = []
        for (c0, cw) in chunks(nq - 1, KC):
            cur += qk_tiles(nq - 1, c0, cw)
        for i in range(QDELAY - 1, -1, -1):
            qpiece(blk(i))
        unpack_weights(next_slot, odd=not odd)
        mb = rowmax(cur)

        for i in range(nq - 1, -1, -1):
            nxt_chunks = chunks(i - 1, KC) if i > 0 else []
            nxt = []
            l = None
            acc = None
            prev_o = None
            ci = 0
            pv_chunks = chunks(i, PVC)
            npv = len(pv_chunks)
            for pi, (c0, cw) in enumerate(pv_chunks):
                mbc = mb if prev_o is None else mb + prev_o * 0.0
                ps = [jnp.exp2(cur[t] - mbc) for t in range(c0 // 128, (c0 + cw) // 128)]
                pj = ps[0] if len(ps) == 1 else jnp.concatenate(ps, axis=1)
                psum = ps[0]
                for p in ps[1:]:
                    psum = psum + p
                l = psum if l is None else l + psum
                o = _dot(pj.astype(bf16), v_s[c0:c0 + cw, :])
                prev_o = o
                acc = o if acc is None else acc + o
                while ci < len(nxt_chunks) and ci * npv < (pi + 1) * len(nxt_chunks):
                    nxt += qk_tiles(i - 1, *nxt_chunks[ci])
                    ci += 1
                for _ in range(-(-len(pending) // (npv - pi))):
                    pending.pop(0)()
            l = jnp.sum(l, axis=-1, keepdims=True)
            r = pl.reciprocal(l, approx=True)
            r = r * (2.0 - l * r)
            ctx = (acc * r).astype(bf16)
            acc_s[blk(i), :] = acc_s[blk(i), :] + _dot(ctx, wo_s[gs, (D if odd else 0):(2 * D if odd else D), :])
            pending.append(lambda i=i: kpiece(blk(i)))
            if i >= QDELAY:
                pending.append(lambda i=i: qpiece(blk(i)))
            if i >= VDELAY:
                pending.append(lambda i=i: vpiece(blk(i)))
            if nxt:
                cur = nxt
                mb = rowmax(cur)
        while pending:
            pending.pop(0)()

    G = H // 2

    def two_heads(g, carry):
        gs = g % 2
        wocopy(g, gs).wait()
        wocopy(jnp.minimum(g + 1, G - 1), 1 - gs).start()
        head_body(gs, False, gs)
        for cp in pcopies(jnp.minimum(g + 1, G - 1), 1 - gs):
            cp.wait()
        for cp in pcopies(jnp.minimum(g + 2, G - 1), gs):
            cp.start()
        head_body(gs, True, 1 - gs)
        return carry

    lax.fori_loop(0, G, two_heads, 0)
    wocopy(G - 1, G % 2).wait()
    for cp in pcopies(G - 1, (G - 1) % 2):
        cp.wait()

    cp_wmod1.wait()
    cp_w1.wait()
    cp_w2.wait()
    cp_w3.wait()
    cp_w4.wait()
    ga, sb, cb, gb = (_dot(sc16, wmod_s[:, j * M:(j + 1) * M])[0:1, :] for j in range(2, 6))

    for k in range(S // SB):
        r = slice(k * SB, (k + 1) * SB)
        x2 = x_s[r, :].astype(f32) + ga * acc_s[r, :]
        x2_s[r, :] = x2
        hb = _ln(x2) * (1.0 + cb) + sb
        h_s[r, :] = hb
        h1_s[k * SB + 8:(k + 1) * SB + 8, :] = _gelu(_dot(_ln(hb).astype(bf16), w1_s[...]))

    lane = lax.broadcasted_iota(jnp.int32, (SB, 128), 1)

    def mix(r0):
        r = pl.ds(r0, SB)
        win = h1_s[pl.ds(r0, SB + 16), :]

        def sh(off, t):
            return win[8 + off:8 + off + SB, t * 128:(t + 1) * 128]

        t0 = sh(-1, 0)
        t1 = jnp.where(lane < 32, sh(-1, 1), sh(1, 1))
        t2 = jnp.where(lane < 64, sh(1, 2), sh(-2, 2))
        t3 = jnp.where(lane < 96, sh(-2, 3), sh(2, 3))
        t4 = sh(2, 4)
        g = jnp.concatenate([t0, t1, t2, t3, t4], axis=1).astype(bf16)
        x1 = h_s[r, :] + _dot(g, w2_s[...])
        y = x2_s[r, :] + gb * x1
        return y, _ln(x1).astype(bf16)

    def mlp(r0, y, ln1):
        r = pl.ds(r0, SB)
        u = _gelu(_dot_nt(ln1, w3t_s[...])).astype(bf16)
        out_s[r, :] = (y + gb * _dot(u, w4_s[...])).astype(bf16)
        pltpu.make_async_copy(out_s.at[r, :], out_hbm.at[r, :], sems.at[6]).start()

    def pass2(i, carry):
        base = pl.multiple_of(i * RB, RB)
        starts = [pl.multiple_of(base + k * SB, SB) for k in range(RB // SB)]
        staged = [mix(r0) for r0 in starts]
        for r0, (y, ln1) in zip(starts, staged):
            mlp(r0, y, ln1)
        return carry

    lax.fori_loop(0, S // RB, pass2, 0)
    cp_out.wait()


@jax.jit
def pallas_adaLN_cond__compressed_kv_cla__mixer_s_mlp__prompt_kernel(
        A_x, A_c_kv, A_w_q, A_w_uk, A_w_uv, A_w_o, B_x, B_w1, B_w2, B_w3, B_w4, c, w_mod):
    del B_x
    hbm = pl.BlockSpec(memory_space=pltpu.HBM)
    out = pl.pallas_call(
        _kernel,
        in_specs=[hbm] * 12,
        out_specs=hbm,
        out_shape=jax.ShapeDtypeStruct((S, M), bf16),
        scratch_shapes=[
            pltpu.VMEM((S, M), bf16),
            pltpu.VMEM((S, DC), bf16),
            pltpu.VMEM((1, M), bf16),
            pltpu.VMEM((S, M), bf16),
            pltpu.VMEM((M, 6 * M), bf16),
            pltpu.VMEM((2, 2 * D, M), bf16),
            pltpu.VMEM((M, M), bf16),
            pltpu.VMEM((M, M), bf16),
            pltpu.VMEM((FP, M), bf16),
            pltpu.VMEM((FP, M), bf16),
            pltpu.VMEM((M, D), bf16),
            pltpu.VMEM((DC, D), bf16),
            pltpu.VMEM((DC, D), bf16),
            pltpu.VMEM((2, M, D), u32),
            pltpu.VMEM((2, DC, D), u32),
            pltpu.VMEM((2, DC, D), u32),
            pltpu.VMEM((S, D), bf16),
            pltpu.VMEM((S, D), bf16),
            pltpu.VMEM((S, D), bf16),
            pltpu.VMEM((S, M), f32),
            pltpu.VMEM((S, M), f32),
            pltpu.VMEM((S, M), f32),
            pltpu.VMEM((S + 16, M), f32),
            pltpu.VMEM((S, M), bf16),
            pltpu.SemaphoreType.DMA((8,)),
            pltpu.SemaphoreType.DMA((4, 2)),
            pltpu.SemaphoreType.DMA((2, S // PB)),
        ],
        compiler_params=pltpu.CompilerParams(
            vmem_limit_bytes=100 * 1024 * 1024,
            flags={"XLA_TPU_RESCHEDULE_DMA_DONES": True},
        ),
    )(A_x.reshape(S, M), A_c_kv.reshape(S, DC), A_w_q, A_w_uk, A_w_uv, A_w_o.reshape(H * D, M),
      B_w1, B_w2, B_w3.T, B_w4, c, w_mod)
    return out.reshape(1, S, M)
```
